```python
import os as _os
_os.environ.setdefault('JAX_PLATFORMS', 'cpu')
import jax
import jax.numpy as jnp

def _softmax(x, axis=-1):
    return jax.nn.softmax(x, axis=axis)

def _gelu(x):
    return jax.nn.gelu(x, approximate=True)

def _silu(x):
    return jax.nn.silu(x)

def _sigmoid(x):
    return jax.nn.sigmoid(x)

def _layernorm(x, axis=-1, eps=1e-05):
    m = jnp.mean(x, axis=axis, keepdims=True)
    v = jnp.var(x, axis=axis, keepdims=True)
    return (x - m) / jnp.sqrt(v + eps)

def _scatter_add(tgt, idx, src, axis=0):
    return tgt.at[idx].add(src)

def _segment_sum(src, seg, n):
    return jax.ops.segment_sum(src, seg, n)

class _Rng:

    def __init__(self, key):
        self._k = key

    def _next(self):
        self._k, sub = jax.random.split(self._k)
        return sub

    def normal(self, shape):
        return jax.random.normal(self._next(), shape, dtype=jnp.bfloat16)

    def randint(self, lo, hi, shape):
        return jax.random.randint(self._next(), shape, lo, hi, dtype=jnp.int32)

    def uniform(self, shape, lo=0.0, hi=1.0):
        return jax.random.uniform(self._next(), shape, jnp.bfloat16, lo, hi)

    def permutation(self, n):
        return jax.random.permutation(self._next(), n)
kernel_name = 'gated_mix__ssm_conv_h3__memory_aug_recurrent_mem_tr__prompt'

def setup_inputs():
    _rng = _Rng(jax.random.key(int.from_bytes(__import__("os").urandom(4), "little")))
    _w = lambda a: (lambda t: t.astype(jnp.bfloat16) if jnp.issubdtype(t.dtype, jnp.floating) else t)(jnp.asarray(a))

    def _A_setup():
        B, S, D = (1, 2048, 1024)
        ks = 4
        return {'q': _w((lambda *s: _rng.normal(s) * 0.05)(B, S, D)), 'k': _w((lambda *s: _rng.normal(s) * 0.4)(B, S, D)), 'v': _w((lambda *s: _rng.normal(s) * 0.4)(B, S, D)), 'shift_k': _w((lambda *s: _rng.normal(s) * 0.4)(D, ks) * 0.5), 'ssm_k': _w((lambda *s: _rng.normal(s) * 0.4)(D, S) * (1.0 / S ** 0.5)), 'ssm_D': _w((lambda *s: _rng.normal(s) * 0.4)(D))}
    _A_in = _A_setup()

    def _B_setup():
        B, S, Dm = (1, 2048, 1024)
        H, Dh = (32, 128)
        M, seg = (8, 32)
        seg = min(seg, S)
        S = S // seg * seg
        return {'x': _w((lambda *s: _rng.normal(s) * 0.05)(B, S, Dm)), 'mem0': _w((lambda *s: _rng.normal(s) * 0.4)(B, M, Dm)), 'Wq': _w((lambda *s: _rng.normal(s) * 3.2)(Dm, H, Dh) * Dm ** (-0.5)), 'Wk': _w((lambda *s: _rng.normal(s) * 3.2)(Dm, H, Dh) * Dm ** (-0.5)), 'Wv': _w((lambda *s: _rng.normal(s) * 0.4)(Dm, H, Dh) * Dm ** (-0.5)), 'Wo': _w((lambda *s: _rng.normal(s) * 0.4)(H, Dh, Dm) * (H * Dh) ** (-0.5)), 'seg_len': seg}
    _B_in = _B_setup()
    return {'A_q': _A_in['q'], 'A_k': _A_in['k'], 'A_v': _A_in['v'], 'A_shift_k': _A_in['shift_k'], 'A_ssm_k': _A_in['ssm_k'], 'A_ssm_D': _A_in['ssm_D'], 'B_x': _B_in['x'], 'B_mem0': _B_in['mem0'], 'B_Wq': _B_in['Wq'], 'B_Wk': _B_in['Wk'], 'B_Wv': _B_in['Wv'], 'B_Wo': _B_in['Wo'], 'B_seg_len': _B_in['seg_len'], 'gate_w': _w((lambda *s: _rng.normal(s) * 0.05)(1024) * 16.0)}

def reference(A_q, A_k, A_v, A_shift_k, A_ssm_k, A_ssm_D, B_x, B_mem0, B_Wq, B_Wk, B_Wv, B_Wo, B_seg_len, gate_w):

    def _A_ref(q, k, v, shift_k, ssm_k, ssm_D):
        B, S, D = q.shape
        ks = shift_k.shape[-1]
        k_pad = jnp.pad(k, ((0, 0), (ks - 1, 0), (0, 0)))
        k_shift = jnp.zeros_like(k)
        for t in range(ks):
            k_shift = k_shift + k_pad[:, t:t + S, :] * shift_k[:, ks - 1 - t][None, None, :]
        kv = k_shift * v
        L = 2 * S
        kv_pad = jnp.pad(kv, ((0, 0), (0, S), (0, 0)))
        kf_pad = jnp.pad(ssm_k, ((0, 0), (0, S)))
        kv_f = (lambda x, axes=(-2, -1): jnp.fft.rfft2(x.astype(jnp.float32), axes=axes))(kv_pad[:, None, :, :], axes=(1, 2))
        kf_f = (lambda x, axes=(-2, -1): jnp.fft.rfft2(x.astype(jnp.float32), axes=axes))(kf_pad[:, None, :], axes=(1, 2))
        kf_f = (lambda x, *d: x.transpose(*d))(kf_f, 1, 2, 0)
        y_f = kv_f * kf_f[None, :, :, :]
        y = (lambda x, s, axes=(-2, -1): jnp.fft.irfft2(x, s=s, axes=axes).astype(jnp.bfloat16))(y_f, (1, L), axes=(1, 2))[:, 0, :S, :]
        y = y + kv * ssm_D[None, None, :]
        return q * y

    def _B_ref(x, mem0, Wq, Wk, Wv, Wo, seg_len):
        B, S, Dm = x.shape
        H, Dh = (Wq.shape[1], Wq.shape[2])
        M = mem0.shape[1]
        scale = Dh ** (-0.5)
        n_seg = S // seg_len
        L = M + seg_len
        idx = jnp.arange(L)
        mask = (idx[:, None] < M) | (idx[:, None] >= idx[None, :])
        mem = mem0
        outs = []
        for s in range(n_seg):
            xs = x[:, s * seg_len:(s + 1) * seg_len, :].copy()
            h = jnp.concatenate([mem, xs], axis=1)
            q = jnp.einsum('btd,dhe->bhte', h, Wq)
            k = jnp.einsum('btd,dhe->bhte', h, Wk)
            v = jnp.einsum('btd,dhe->bhte', h, Wv)
            scores = jnp.einsum('bhqe,bhke->bhqk', q, k) * scale
            scores = jnp.where(mask[None, None], scores, -1000000000.0)
            p = _softmax(scores, axis=-1)
            o = jnp.einsum('bhqk,bhke->bhqe', p, v)
            o = jnp.einsum('bhte,hed->btd', o, Wo)
            mem = o[:, :M, :].copy()
            outs.append(o[:, M:, :])
        return jnp.concatenate(outs, axis=1)
    x = A_q
    g = _sigmoid((x * gate_w).sum(-1, keepdims=True))
    a = _A_ref(x, A_k, A_v, A_shift_k, A_ssm_k, A_ssm_D)
    b = _B_ref(x, B_mem0, B_Wq, B_Wk, B_Wv, B_Wo, B_seg_len)
    return g * a + (1 - g) * b
```

```python
import functools

import jax
import jax.numpy as jnp
import numpy as np
from jax import lax
import jax.experimental.pallas as pl
import jax.experimental.pallas.tpu as pltpu

f32, bf16, u32 = jnp.float32, jnp.bfloat16, jnp.uint32

S, D, H, E, M, SEG, KS = 2048, 1024, 32, 128, 8, 32, 4
NP = S // (2 * SEG)
NC = D // 128
NB = S // 128
SCALE = float(E) ** -0.5
NEG = -1000000000.0
D1, D2, HB = 1, 2, 4


def _pack_rows(a):
    b = np.asarray(a, np.float32).astype(jnp.bfloat16).view(np.uint16).astype(np.uint32)
    return b[0::2] | (b[1::2] << 16)


def _dft_consts():
    t = np.arange(128, dtype=np.float64)
    f = np.arange(128, dtype=np.float64) + 0.5
    th = 2.0 * np.pi * np.outer(f, t) / 256.0
    fwd = np.concatenate([np.cos(th), -np.sin(th)], axis=0)
    inv = np.concatenate([np.cos(th).T, -np.sin(th).T], axis=1) / 128.0
    return _pack_rows(fwd), _pack_rows(inv)


def _b(x):
    return pltpu.bitcast(x, bf16)


def _u(x):
    return pltpu.bitcast(x, u32)


def _dot(a, b):
    return jnp.dot(a, b, preferred_element_type=f32)


def _dot_t(a, b):
    return lax.dot_general(a, b, (((1,), (1,)), ((), ())), preferred_element_type=f32)


def _kernel(x_hbm, k_hbm, v_hbm, ssm_hbm, wq_hbm, wk_hbm, wv_hbm, wo_hbm,
            shift_ref, ssmd_ref, gate_ref, mem0_ref, fwd_ref, inv_ref,
            out_hbm,
            x_v, xb_v, xbp, k_v, v_v, ssm_v, wraw, woraw, w_s, wo_s, bulk,
            ys, kpad, kvb, uh, kh, zz, mem_sc, kv_sc, oall, out_v,
            sem_c, sem_x, sem_w, sem_o, sem_out):
    def conv_copies(c):
        return (
            pltpu.make_async_copy(k_hbm.at[:, pl.ds(c * 128, 128)], k_v.at[c], sem_c.at[c, 0]),
            pltpu.make_async_copy(v_hbm.at[:, pl.ds(c * 128, 128)], v_v.at[c], sem_c.at[c, 1]),
            pltpu.make_async_copy(ssm_hbm.at[pl.ds(c * 128, 128), :], ssm_v.at[c], sem_c.at[c, 2]),
        )

    xb_cp = pltpu.make_async_copy(x_hbm.at[:, pl.ds(24, 16), :], xb_v, sem_x.at[0])
    x_cp = pltpu.make_async_copy(x_hbm, x_v, sem_x.at[1])
    w_cps = [pltpu.make_async_copy(w, wraw.at[i], sem_w.at[i])
             for i, w in enumerate((wq_hbm, wk_hbm, wv_hbm))]
    wo_cps = [pltpu.make_async_copy(wo_hbm.at[:, pl.ds(j * 128, 128)], woraw.at[j], sem_o.at[j])
              for j in range(NC)]

    for c in range(NC):
        for cp in conv_copies(c):
            cp.start()
    xb_cp.start()
    for cp in w_cps:
        cp.start()
    for cp in wo_cps:
        cp.start()
    x_cp.start()

    kpad[0:8, :] = jnp.zeros((8, 128), f32)
    sgn = jnp.where(lax.broadcasted_iota(jnp.int32, (128, 128), 0) % 2 == 0, 1.0, -1.0).astype(f32)

    def conv_tile(c):
        fwd = _b(fwd_ref[...])
        inv = _b(inv_ref[...])
        sh = shift_ref[c]
        dvec = ssmd_ref[c]
        for i in range(NB):
            kpad[8 + 128 * i:8 + 128 * (i + 1), :] = k_v[c, 128 * i:128 * (i + 1), :].astype(f32)
        prev_r = prev_i = None
        for i in range(NB):
            ks = kpad[8 + 128 * i:8 + 128 * (i + 1), :] * sh[0:1, :]
            for j in range(1, KS):
                ks = ks + kpad[8 + 128 * i - j:8 + 128 * (i + 1) - j, :] * sh[j:j + 1, :]
            kv = (ks * v_v[c, 128 * i:128 * (i + 1), :].astype(f32)).astype(bf16)
            kvb[64 * i:64 * (i + 1), :] = _u(kv)
            u = _dot(fwd, kv)
            ur, ui = u[:128], u[128:]
            uh[0, i] = ur
            uh[1, i] = ui
            uh[2, i] = ur + ui
            kk = _dot_t(fwd, ssm_v[c, :, 128 * i:128 * (i + 1)])
            kr, ki = kk[:128], kk[128:]
            if i == 0:
                pr, pi = kr, ki
            else:
                pr = kr - sgn * prev_i
                pi = ki + sgn * prev_r
            prev_r, prev_i = kr, ki
            kh[0, i] = pr
            kh[1, i] = pi
            kh[2, i] = pr + pi

        def blockconv(comp, p):
            uu = uh[comp, :, 8 * p:8 * (p + 1), :]
            acc = uu * kh[comp, 0, 8 * p:8 * (p + 1), :][None]
            for m in range(1, NB):
                t = uu[:NB - m] * kh[comp, m, 8 * p:8 * (p + 1), :][None]
                acc = jnp.concatenate([acc[:m], acc[m:] + t], axis=0)
            return acc

        for p in range(16):
            a = blockconv(0, p)
            b = blockconv(1, p)
            zz[:, 8 * p:8 * (p + 1), :] = a - b
            ab = a + b
            cc = blockconv(2, p)
            zz[:, 128 + 8 * p:128 + 8 * (p + 1), :] = cc - ab
        for i in range(NB):
            y = _dot(inv, zz[i].astype(bf16))
            kv = _b(kvb[64 * i:64 * (i + 1), :]).astype(f32)
            yy = y.astype(bf16).astype(f32) + kv * dvec
            ys[c, 128 * i:128 * (i + 1), :] = yy

    def conv_body(c, carry):
        for cp in conv_copies(c):
            cp.wait()
        conv_tile(c)
        return carry

    lax.fori_loop(0, NC, conv_body, 0)

    wraw32 = wraw.bitcast(u32)
    for i in range(3):
        w_cps[i].wait()

        def relayout(db, carry, i=i):
            d0 = pl.multiple_of(db * 128, 128)
            blk = wraw32.at[i, pl.ds(pl.multiple_of(db * 2048, 2048), 2048), :]
            for j in range(H // 2):
                a = blk[pl.ds(j, 128, stride=16), :]
                lo = pltpu.bitcast(a << 16, f32).astype(bf16)
                hi = pltpu.bitcast(a & jnp.uint32(0xFFFF0000), f32).astype(bf16)
                r0 = pl.multiple_of(db * 64, 64)
                w_s[i * H + 2 * j, pl.ds(r0, 64), :] = _u(lo)
                w_s[i * H + 2 * j + 1, pl.ds(r0, 64), :] = _u(hi)
            return carry

        lax.fori_loop(0, D // 128, relayout, 0)

    xb_cp.wait()
    for j in range(NP):
        xbp[8 * j:8 * (j + 1), :] = _u(xb_v[j])

    def bulk_body(u, carry):
        w = _b(w_s[u])
        for mc in range(4):
            r = _dot(_b(xbp[64 * mc:64 * (mc + 1), :]), w)
            bulk[u, 64 * mc:64 * (mc + 1), :] = _u(r.astype(bf16))
        return carry

    lax.fori_loop(0, 3 * H, bulk_body, 0)

    for j in range(NC):
        wo_cps[j].wait()

        def repack(rb, carry, j=j):
            wo_s[j, pl.ds(pl.multiple_of(rb * 256, 256), 256), :] = _u(
                woraw[j, pl.ds(pl.multiple_of(rb * 512, 512), 512), :])
            return carry

        lax.fori_loop(0, 8, repack, 0)
    x_cp.wait()

    mem_sc[...] = mem0_ref[...].astype(f32)

    ra = lax.broadcasted_iota(jnp.int32, (32, 48), 0)
    ca = lax.broadcasted_iota(jnp.int32, (32, 48), 1)
    mask_a = (ca < 40) & ((ra < M) | (ra >= ca))
    rb_ = lax.broadcasted_iota(jnp.int32, (48, 80), 0)
    cb_ = lax.broadcasted_iota(jnp.int32, (48, 80), 1)
    q_in_a = (rb_ >= 32) & (rb_ < 40)
    k_in_a = ((cb_ >= 32) & (cb_ < 40)) | (cb_ >= 48)
    qpos = jnp.where(rb_ < 8, rb_, jnp.where(rb_ < 32, rb_ + 8, jnp.where(rb_ < 40, rb_, rb_ - 32)))
    kpos = jnp.where(cb_ < 8, cb_, jnp.where(cb_ < 32, cb_ + 8,
                     jnp.where(cb_ < 40, cb_, jnp.where(cb_ < 48, cb_ - 32, cb_ - 48))))
    mask_b = (q_in_a == k_in_a) & ((qpos < M) | (qpos >= kpos))

    def step(first, jp):
        mem = mem_sc[...]
        if first:
            xr = x_v[jp, 0:24, :].astype(f32)
        else:
            xr = x_v[jp, 40:64, :].astype(f32)
        lhs = jnp.concatenate([mem, xr], axis=0).astype(bf16)
        nw = 32 if first else 48
        mask = mask_a if first else mask_b
        br = pl.ds(pl.multiple_of(jp * 8, 8), 8)
        qkv, ps = {}, {}

        def proj(h):
            q = _dot(lhs, _b(w_s[h])).astype(bf16)
            k = _dot(lhs, _b(w_s[H + h])).astype(bf16)
            v = _dot(lhs, _b(w_s[2 * H + h])).astype(bf16)
            kb = _b(bulk[H + h, br, :])
            vb = _b(bulk[2 * H + h, br, :])
            if first:
                kv_sc[0, h] = _u(k)
                kv_sc[1, h] = _u(v)
                k = jnp.concatenate([k, kb], axis=0)
                v = jnp.concatenate([v, vb], axis=0)
            else:
                q = jnp.concatenate([q, _b(bulk[h, br, :])], axis=0)
                k = jnp.concatenate([k, kb, _b(kv_sc[0, h])], axis=0)
                v = jnp.concatenate([v, vb, _b(kv_sc[1, h])], axis=0)
            qkv[h] = (q, k, v)

        def qk(h):
            q, k, _ = qkv[h]
            s = jnp.where(mask, _dot_t(q, k) * SCALE, NEG)
            m = jnp.max(s, axis=-1, keepdims=True)
            p = jnp.exp(s - m)
            den = jnp.sum(p, axis=-1, keepdims=True)
            ps[h] = (p * pl.reciprocal(den, approx=False)).astype(bf16)

        def pv(h):
            o = _dot(ps.pop(h), qkv.pop(h)[2])
            oall[0:nw // 2, h * 128:(h + 1) * 128] = _u(o.astype(bf16))

        for h in range(H):
            proj(h)
            if h - D1 >= 0:
                qk(h - D1)
            if h - D1 - D2 >= 0:
                pv(h - D1 - D2)

        ka = (H - HB) * 128
        pend = []
        for t in range(H, H + D1 + D2):
            ops = []
            if t - D1 < H:
                ops.append((qk, t - D1))
            ops.append((pv, t - D1 - D2))
            pend.append(ops)
        oa = _b(oall[0:nw // 2, 0:ka])
        accs = []
        sched = [2, 2, 2, 2]
        assert len(pend) == 3
        for i, n in enumerate(sched):
            for _ in range(n):
                accs.append(_dot(oa, _b(wo_s[len(accs), 0:ka // 2, :])))
            if i < len(pend):
                for fn, hh in pend[i]:
                    fn(hh)
        ob = _b(oall[0:nw // 2, ka:])
        res = [_dot(ob, _b(wo_s[j, ka // 2:, :])) + accs[j] for j in range(NC)]

        mem_sc[...] = jnp.concatenate([r[:M] for r in res], axis=1).astype(bf16).astype(f32)

        if first:
            lo, n = 0, 24
            xo = xr
        else:
            lo, n = 24, 40
            xo = jnp.concatenate([x_v[jp, 24:40, :].astype(f32), xr], axis=0)
        g = jax.nn.sigmoid(jnp.sum(xo * gate_ref[...], axis=-1, keepdims=True))
        row0 = pl.multiple_of(jp * 64, 64) + lo
        for j in range(NC):
            if first:
                bj = res[j][8:32]
            else:
                bj = jnp.concatenate([res[j][32:48], res[j][8:32]], axis=0)
            aj = xo[:, j * 128:(j + 1) * 128] * ys[j, pl.ds(pl.multiple_of(row0, 8), n), :]
            out_v[jp, lo:lo + n, j * 128:(j + 1) * 128] = (g * aj + (1.0 - g) * bj).astype(bf16)

    def out_copy(jp):
        return pltpu.make_async_copy(out_v.at[jp], out_hbm.at[jp], sem_out)

    def pair(jp, carry):
        step(True, jp)
        step(False, jp)
        out_copy(jp).start()
        return carry

    lax.fori_loop(0, NP, pair, 0)
    pltpu.make_async_copy(out_v, out_hbm, sem_out).wait()


@functools.partial(jax.jit, static_argnames=("B_seg_len",))
def pallas_gated_mix__ssm_conv_h3__memory_aug_recurrent_mem_tr__prompt_kernel(
    A_q, A_k, A_v, A_shift_k, A_ssm_k, A_ssm_D, B_x, B_mem0, B_Wq, B_Wk, B_Wv, B_Wo,
    B_seg_len, gate_w,
):
    del B_x
    assert int(B_seg_len) == SEG and A_q.shape == (1, S, D)
    fwd, inv = _dft_consts()
    shift = jnp.pad(A_shift_k.astype(f32).T, ((0, 8 - KS), (0, 0)))
    shift = shift.reshape(8, NC, 128).transpose(1, 0, 2)
    ssmd = A_ssm_D.astype(f32).reshape(NC, 1, 128)
    gate = gate_w.astype(f32).reshape(1, D)

    any_spec = pl.BlockSpec(memory_space=pl.ANY)
    vmem_spec = pl.BlockSpec(memory_space=pltpu.VMEM)
    out = pl.pallas_call(
        _kernel,
        out_shape=jax.ShapeDtypeStruct((NP, 64, D), bf16),
        in_specs=[any_spec] * 8 + [vmem_spec] * 6,
        out_specs=any_spec,
        scratch_shapes=[
            pltpu.VMEM((NP, 64, D), bf16),
            pltpu.VMEM((NP, 16, D), bf16),
            pltpu.VMEM((NP * 8, D), u32),
            pltpu.VMEM((NC, S, 128), bf16),
            pltpu.VMEM((NC, S, 128), bf16),
            pltpu.VMEM((NC, 128, S), bf16),
            pltpu.VMEM((3, D * H, E), bf16),
            pltpu.VMEM((NC, H * E, 128), bf16),
            pltpu.VMEM((3 * H, D // 2, E), u32),
            pltpu.VMEM((NC, H * E // 2, 128), u32),
            pltpu.VMEM((3 * H, NP * 8, E), u32),
            pltpu.VMEM((NC, S, 128), f32),
            pltpu.VMEM((S + 8, 128), f32),
            pltpu.VMEM((S // 2, 128), u32),
            pltpu.VMEM((3, NB, 128, 128), f32),
            pltpu.VMEM((3, NB, 128, 128), f32),
            pltpu.VMEM((NB, 256, 128), f32),
            pltpu.VMEM((M, D), f32),
            pltpu.VMEM((2, H, 16, E), u32),
            pltpu.VMEM((24, H * E), u32),
            pltpu.VMEM((NP, 64, D), bf16),
            pltpu.SemaphoreType.DMA((NC, 3)),
            pltpu.SemaphoreType.DMA((2,)),
            pltpu.SemaphoreType.DMA((3,)),
            pltpu.SemaphoreType.DMA((NC,)),
            pltpu.SemaphoreType.DMA,
        ],
        compiler_params=pltpu.CompilerParams(vmem_limit_bytes=126 * 1024 * 1024),
    )(
        A_q.reshape(NP, 64, D), A_k.reshape(S, D), A_v.reshape(S, D), A_ssm_k,
        B_Wq.reshape(D * H, E), B_Wk.reshape(D * H, E), B_Wv.reshape(D * H, E),
        B_Wo.reshape(H * E, D),
        shift, ssmd, gate, B_mem0.reshape(M, D), jnp.asarray(fwd), jnp.asarray(inv),
    )
    return out.reshape(1, S, D)
```

```python
import functools

import jax
import jax.numpy as jnp
import numpy as np
from jax import lax
import jax.experimental.pallas as pl
import jax.experimental.pallas.tpu as pltpu

f32, bf16, u32 = jnp.float32, jnp.bfloat16, jnp.uint32

S, D, H, E, M, SEG, KS = 2048, 1024, 32, 128, 8, 32, 4
NP = S // (2 * SEG)
NC = D // 128
NB = S // 128
NW = 3 * H // 2
SCALE = float(E) ** -0.5
NEG = -1000000000.0
D1, D2, HB = 2, 2, 5
KSPLIT = 2
UN = 2
MB = 64


def _pack_rows(a):
    b = np.asarray(a, np.float32).astype(jnp.bfloat16).view(np.uint16).astype(np.uint32)
    return b[0::2] | (b[1::2] << 16)


def _dft_consts():
    t = np.arange(128, dtype=np.float64)
    f = np.arange(128, dtype=np.float64) + 0.5
    th = 2.0 * np.pi * np.outer(f, t) / 256.0
    fwd = np.concatenate([np.cos(th), -np.sin(th)], axis=0)
    inv = np.concatenate([np.cos(th).T, -np.sin(th).T], axis=1) / 128.0
    return _pack_rows(fwd), _pack_rows(inv)


def _b(x):
    return pltpu.bitcast(x, bf16)


def _u(x):
    return pltpu.bitcast(x, u32)


def _dot(a, b):
    return jnp.dot(a, b, preferred_element_type=f32)


def _dot_t(a, b):
    return lax.dot_general(a, b, (((1,), (1,)), ((), ())), preferred_element_type=f32)


def _cat(lists):
    return [f for lst in lists for f in lst]


def _interleave(*lists):
    items = []
    for li, lst in enumerate(lists):
        for i, fn in enumerate(lst):
            items.append(((i + 0.5) / len(lst), li, i, fn))
    items.sort(key=lambda t: t[:3])
    for it in items:
        it[3]()


def _kernel(x_hbm, k_hbm, v_hbm, ssm_hbm, wq_hbm, wk_hbm, wv_hbm, wo_hbm,
            shift_hbm, ssmd_hbm, gate_hbm, mem0_hbm, fwd_hbm, inv_hbm,
            out_hbm,
            x_v, xbp, k_v, v_v, ssm_v, wraw, w_s, wo_s, bulk,
            ys, gtab, kpad, kraw, uh, kh, zz, mem_sc, kv_sc, oall, flag,
            shift_v, ssmd_v, gate_v, mem0_ref, fwd_ref, inv_ref, shift_ref, ssmd_ref, gate_ref,
            sem_s, sem_c, sem_x, sem_w, sem_o, sem_out):
    w32 = [w.bitcast(u32) for w in (wq_hbm, wk_hbm, wv_hbm)]
    wo32 = wo_hbm.bitcast(u32)
    x32 = x_hbm.bitcast(u32)

    def tile_copies(c):
        return [
            pltpu.make_async_copy(k_hbm.at[:, pl.ds(c * 128, 128)], k_v.at[c], sem_c.at[c, 0]),
            pltpu.make_async_copy(v_hbm.at[:, pl.ds(c * 128, 128)], v_v.at[c], sem_c.at[c, 1]),
            pltpu.make_async_copy(ssm_hbm.at[pl.ds(c * 128, 128), :], ssm_v.at[c], sem_c.at[c, 2]),
            pltpu.make_async_copy(x_hbm.at[pl.ds(4 * c, 4)], x_v.at[pl.ds(4 * c, 4)], sem_c.at[c, 3]),
        ]

    def w_copies(lo, hi):
        return [pltpu.make_async_copy(w32[t // 16].at[:, par, t % 16, :], wraw.at[t, par], sem_w.at[t])
                for t in range(lo, min(hi, NW)) for par in range(2)]

    def w_wait(t):
        pltpu.make_async_copy(wraw.at[t], wraw.at[t], sem_w.at[t]).wait()

    def wo_copy(j):
        return pltpu.make_async_copy(wo32.at[:, pl.ds(j * 128, 128)], wo_s.at[j], sem_o.at[j])

    def xb_copy():
        return pltpu.make_async_copy(x32.at[:, pl.ds(12, 8), :], xbp, sem_x)

    def small_copies():
        return [pltpu.make_async_copy(a, b, sem_s.at[n]) for n, (a, b) in enumerate(
            ((shift_hbm, shift_v), (ssmd_hbm, ssmd_v), (gate_hbm, gate_v), (mem0_hbm, mem0_ref),
             (fwd_hbm, fwd_ref), (inv_hbm, inv_ref)))]

    def start_all(cps):
        for cp in cps:
            cp.start()

    def wait_all(cps):
        for cp in cps:
            cp.wait()

    def start_head_batch(t):
        start_all({0: lambda: w_copies(4, 8),
                   2: lambda: tile_copies(0) + w_copies(8, 10),
                   4: lambda: w_copies(10, 15),
                   6: lambda: tile_copies(1) + w_copies(15, 20)}[t]())

    def start_late_batch(i):
        cps = tile_copies(i + 2) + w_copies(20 + 5 * i, 25 + 5 * i)
        if i < 4:
            cps += [wo_copy(2 * i), wo_copy(2 * i + 1)]
        start_all(cps)

    def once_if(cond, fn):
        def body(_, carry):
            fn()
            return carry
        lax.fori_loop(0, cond.astype(jnp.int32), body, 0)

    start_all([xb_copy()] + w_copies(0, 4) + small_copies())

    flag[0] = 1
    kpad[0:8, :] = jnp.zeros((8, 128), f32)
    zz[...] = jnp.zeros(zz.shape, f32)
    ys[0] = jnp.zeros((S, 128), f32)

    def fwd_thunks(c, ys_c):
        def cvt(i):
            kpad[8 + 128 * i:8 + 128 * (i + 1), :] = k_v[c, 128 * i:128 * (i + 1), :].astype(f32)

        def fu(i):
            sh = shift_ref[c]
            if i == 0:
                cvt(0)
            if i + 1 < NB:
                cvt(i + 1)
            ks = kpad[8 + 128 * i:8 + 128 * (i + 1), :] * sh[0:1, :]
            for j in range(1, KS):
                ks = ks + kpad[8 + 128 * i - j:8 + 128 * (i + 1) - j, :] * sh[j:j + 1, :]
            kv = (ks * v_v[c, 128 * i:128 * (i + 1), :].astype(f32)).astype(bf16)
            ys_c[128 * i:128 * (i + 1), :] = kv.astype(f32) * ssmd_ref[c]
            u = _dot(_b(fwd_ref[...]), kv)
            ur, ui = u[:128], u[128:]
            uh[0, i] = ur
            uh[1, i] = ui
            uh[2, i] = ur + ui

        def fk(i):
            kk = _dot_t(_b(fwd_ref[...]), ssm_v[c, :, 128 * i:128 * (i + 1)])
            kr, ki = kk[:128], kk[128:]
            if i == 0:
                pr, pi = kr, ki
            else:
                row = lax.broadcasted_iota(jnp.int32, (128, 128), 0)
                sgn = jnp.where(row % 2 == 0, 1.0, -1.0).astype(f32)
                pr = kr - sgn * kraw[1]
                pi = ki + sgn * kraw[0]
            kraw[0] = kr
            kraw[1] = ki
            kh[0, i] = pr
            kh[1, i] = pi
            kh[2, i] = pr + pi

        return _cat([functools.partial(fu, i), functools.partial(fk, i)] for i in range(NB))

    def group4(comp, rows, b):
        acc = None
        for j in range(4 * b + 4):
            lo = max(0, j - 4 * b)
            t = kh[comp, 4 * b + lo - j:4 * b + 4 - j, rows, :] * uh[comp, j, rows, :][None]
            if acc is None:
                acc = t
            elif lo == 0:
                acc = acc + t
            else:
                acc = jnp.concatenate([acc[:lo], acc[lo:] + t], axis=0)
        return acc

    def mac_thunks(p):
        rows, rows2 = pl.ds(8 * p, 8), pl.ds(128 + 8 * p, 8)
        out = []
        for b in range(4):
            st = {}

            def f0(b=b, st=st):
                st['a'] = group4(0, rows, b)

            def f1(b=b, st=st):
                bb = group4(1, rows, b)
                a = st.pop('a')
                zz[4 * b:4 * b + 4, rows, :] = a - bb
                st['ab'] = a + bb

            def f2(b=b, st=st):
                zz[4 * b:4 * b + 4, rows2, :] = group4(2, rows, b) - st.pop('ab')

            out += [f0, f1, f2]
        return out

    def inv_thunks(ys_c):
        def f(i):
            y = _dot(_b(inv_ref[...]), zz[i].astype(bf16))
            ys_c[128 * i:128 * (i + 1), :] = ys_c[128 * i:128 * (i + 1), :] + y.astype(bf16).astype(f32)
        return [functools.partial(f, i) for i in range(NB)]

    def gate_thunks(i):
        def f(r):
            rows = pl.ds(32 * (r % 2), 32)
            xo = x_v[4 * i + r // 2, rows, :].astype(f32)
            g = jax.nn.sigmoid(jnp.sum(xo * gate_ref[...], axis=-1, keepdims=True))
            gtab[4 * i + r // 2, rows, :] = jnp.broadcast_to(g, (32, 128))
        return [functools.partial(f, r) for r in range(8)]

    def repack_thunks(src, dst):
        def f(db):
            r = pl.ds(db * 64, 64)
            ev, od = src[0, r, :], src[1, r, :]
            dst[0, r, :] = (ev & jnp.uint32(0xFFFF)) | (od << 16)
            dst[1, r, :] = (ev >> 16) | (od & jnp.uint32(0xFFFF0000))
        return [functools.partial(f, db) for db in range(8)]

    def bulk_thunks(wsrc, dst):
        def f(mc):
            lhs = xbp[mc * (MB // 16):(mc + 1) * (MB // 16)].reshape(MB // 2, D)
            r = _dot(_b(lhs), _b(wsrc[...]))
            dst[mc * (MB // 2):(mc + 1) * (MB // 2), :] = _u(r.astype(bf16))
        return [functools.partial(f, mc) for mc in range(NP * 16 // MB)]

    w_wait(0)
    _interleave(repack_thunks(wraw.at[0], w_s.at[pl.ds(0, 2)]))
    xb_copy().wait()

    def head(t, carry):
        for c in (0, 2, 4, 6):
            once_if(t == c, functools.partial(start_head_batch, c))
        w_wait(t + 1)
        wwin = w_s.at[pl.ds(t * 2, 4)]
        bwin = bulk.at[pl.ds(t * 2, 2)]

        @pl.when(flag[0] > 0)
        def _():
            _interleave(_cat(bulk_thunks(wwin.at[u], bwin.at[u]) for u in range(2)),
                        repack_thunks(wraw.at[t + 1], wwin.at[pl.ds(2, 2)]))
        return carry

    lax.fori_loop(0, 8, head, 0)
    wait_all(small_copies())
    sh32 = shift_v[...].astype(f32)
    sd32 = ssmd_v[...].reshape(1, D).astype(f32)
    for c in range(NC):
        shift_ref[c] = sh32[:, c * 128:(c + 1) * 128]
        ssmd_ref[c] = sd32[:, c * 128:(c + 1) * 128]
    gate_ref[...] = gate_v[...].reshape(1, D).astype(f32)
    w_wait(9)
    _interleave(repack_thunks(wraw.at[9], w_s.at[pl.ds(18, 2)]))
    wait_all(tile_copies(0))

    def pro(i, carry):
        wwin = w_s.at[pl.ds(16 + i * 10, 14)]
        bwin = bulk.at[pl.ds(16 + i * 10, 10)]
        ywin = ys.at[pl.ds(i, 2)]
        rwin = wraw.at[pl.ds(10 + i * 5, 5)]

        @pl.when(flag[0] > 0)
        def _():
            _interleave(_cat(bulk_thunks(wwin.at[u], bwin.at[u]) for u in range(2)),
                        fwd_thunks(i, ywin.at[1]), inv_thunks(ywin.at[0]), gate_thunks(i))

        for t in range(3):
            w_wait(10 + i * 5 + t)

        @pl.when(i < NC - 1)
        def _():
            for t in range(3, 5):
                w_wait(10 + i * 5 + t)

        for c in range(NC - 2):
            once_if(i == c, functools.partial(start_late_batch, c))

        @pl.when(flag[0] > 0)
        def _():
            _interleave(_cat(bulk_thunks(wwin.at[2 + u], bwin.at[2 + u]) for u in range(8)),
                        _cat(mac_thunks(p) for p in range(16)),
                        _cat(repack_thunks(rwin.at[t], wwin.at[pl.ds(4 + 2 * t, 2)]) for t in range(5)))

        @pl.when(i < NC - 1)
        def _():
            wait_all(tile_copies(jnp.minimum(i + 1, NC - 1)))
        return carry

    lax.fori_loop(0, NC, pro, 0)
    _interleave(inv_thunks(ys.at[NC]))
    wait_all([wo_copy(j) for j in range(NC)])

    mem_sc[...] = mem0_ref[...].astype(f32)

    ra = lax.broadcasted_iota(jnp.int32, (32, 48), 0)
    ca = lax.broadcasted_iota(jnp.int32, (32, 48), 1)
    same_a = ca < 40
    mask_a = same_a & ((ra < M) | (ra >= ca))
    rb = lax.broadcasted_iota(jnp.int32, (48, 80), 0)
    cb = lax.broadcasted_iota(jnp.int32, (48, 80), 1)
    q_in_a = (rb >= 32) & (rb < 40)
    k_in_a = ((cb >= 32) & (cb < 40)) | (cb >= 48)
    qpos = jnp.where(rb < 8, rb, jnp.where(rb < 32, rb + 8, jnp.where(rb < 40, rb, rb - 32)))
    kpos = jnp.where(cb < 8, cb, jnp.where(cb < 32, cb + 8,
                     jnp.where(cb < 40, cb, jnp.where(cb < 48, cb - 32, cb - 48))))
    same_b = q_in_a == k_in_a
    mask_b = same_b & ((qpos < M) | (qpos >= kpos))
    fill_a = jnp.where(same_a, NEG, -jnp.inf).astype(f32)
    fill_b = jnp.where(same_b, NEG, -jnp.inf).astype(f32)

    def step(first, jp, side):
        xr = x_v[jp, 0:24, :] if first else x_v[jp, 40:64, :]
        lhs = jnp.concatenate([mem_sc[...], xr.astype(f32)], axis=0).astype(bf16)
        nw = 32 if first else 48
        mask, fill = (mask_a, fill_a) if first else (mask_b, fill_b)
        br = pl.ds(pl.multiple_of(jp * 8, 8), 8)
        qkv, ps, part = {}, {}, {}

        def proj_lo(h):
            part[h] = [_dot(lhs[:, :D // 2], _b(w_s[t * H + h, 0:D // 4, :])) for t in range(3)]

        def proj(h):
            if h in part:
                low = part.pop(h)
                q, k, v = [(_dot(lhs[:, D // 2:], _b(w_s[t * H + h, D // 4:, :])) + low[t]).astype(bf16)
                           for t in range(3)]
            else:
                q, k, v = [_dot(lhs, _b(w_s[t * H + h])).astype(bf16) for t in range(3)]
            kb = _b(bulk[H + h, br, :])
            vb = _b(bulk[2 * H + h, br, :])
            if first:
                kv_sc[0, h] = _u(k)
                kv_sc[1, h] = _u(v)
                k = jnp.concatenate([k, kb], axis=0)
                v = jnp.concatenate([v, vb], axis=0)
            else:
                q = jnp.concatenate([q, _b(bulk[h, br, :])], axis=0)
                k = jnp.concatenate([k, kb, _b(kv_sc[0, h])], axis=0)
                v = jnp.concatenate([v, vb, _b(kv_sc[1, h])], axis=0)
            qkv[h] = (q, k, v)

        def qk(h):
            q, k, _ = qkv[h]
            s = jnp.where(mask, _dot_t(q, k) * SCALE, fill)
            p = jnp.exp(s - jnp.max(s, axis=-1, keepdims=True))
            den = jnp.sum(p, axis=-1, keepdims=True)
            ps[h] = (p * pl.reciprocal(den, approx=False)).astype(bf16)

        def pv(h):
            o = _dot(ps.pop(h), qkv.pop(h)[2])
            oall[0:nw // 2, h * 128:(h + 1) * 128] = _u(o.astype(bf16))

        side = list(side)
        for h in range(KSPLIT):
            proj_lo(h)
        for h in range(H):
            proj(h)
            if h - D1 >= 0:
                qk(h - D1)
            if h - D1 - D2 >= 0:
                pv(h - D1 - D2)
            if side and h >= 4 and h % 2 == 0:
                side.pop(0)()

        ka = (H - HB) * 128
        oa = _b(oall[0:nw // 2, 0:ka])
        accs = []
        nslot = D1 + D2 + 1
        for i in range(nslot):
            while len(accs) < (NC * (i + 1)) // nslot:
                accs.append(_dot(oa, _b(wo_s[len(accs), 0:ka // 2, :])))
            if i < D1:
                qk(H + i - D1)
            if i < D1 + D2:
                pv(H + i - D1 - D2)
        ob = _b(oall[0:nw // 2, ka:])
        res = [_dot(ob, _b(wo_s[j, ka // 2:, :])) + accs[j] for j in range(NC)]

        mem_sc[...] = jnp.concatenate([r[:M] for r in res], axis=1).astype(bf16).astype(f32)

        lo, n = (0, 24) if first else (24, 40)

        def mix(j):
            if first:
                bj = res[j][8:32]
            else:
                bj = jnp.concatenate([res[j][32:48], res[j][8:32]], axis=0)
            cols = slice(j * 128, (j + 1) * 128)
            aj = x_v[jp, lo:lo + n, cols].astype(f32) * ys[j + 1, pl.ds(pl.multiple_of(jp * 64 + lo, 8), n), :]
            x_v[jp, lo:lo + n, cols] = (bj + gtab[jp, lo:lo + n, :] * (aj - bj)).astype(bf16)

        return [functools.partial(mix, j) for j in range(NC)]

    def pairs(jq, carry):
        epi = []
        for r in range(UN):
            for first in (True, False):
                epi = step(first, jq * UN + r, epi)
        _interleave(epi)
        rows = pl.ds(jq * UN, UN)
        pltpu.make_async_copy(x_v.at[rows], out_hbm.at[rows], sem_out).start()
        return carry

    lax.fori_loop(0, NP // UN, pairs, 0)
    pltpu.make_async_copy(x_v, out_hbm, sem_out).wait()


@functools.partial(jax.jit, static_argnames=("B_seg_len",))
def pallas_gated_mix__ssm_conv_h3__memory_aug_recurrent_mem_tr__prompt_kernel(
    A_q, A_k, A_v, A_shift_k, A_ssm_k, A_ssm_D, B_x, B_mem0, B_Wq, B_Wk, B_Wv, B_Wo,
    B_seg_len, gate_w,
):
    del B_x
    assert int(B_seg_len) == SEG and A_q.shape == (1, S, D) and B_Wq.shape == (D, H, E)
    fwd, inv = _dft_consts()
    out = pl.pallas_call(
        _kernel,
        out_shape=jax.ShapeDtypeStruct((NP, 64, D), bf16),
        in_specs=[pl.BlockSpec(memory_space=pl.ANY)] * 14,
        out_specs=pl.BlockSpec(memory_space=pl.ANY),
        scratch_shapes=[
            pltpu.VMEM((NP, 64, D), bf16),
            pltpu.VMEM((NP, 8, D), u32),
            pltpu.VMEM((NC, S, 128), bf16),
            pltpu.VMEM((NC, S, 128), bf16),
            pltpu.VMEM((NC, 128, S), bf16),
            pltpu.VMEM((NW + 2, 2, D // 2, E), u32),
            pltpu.VMEM((3 * H + 4, D // 2, E), u32),
            pltpu.VMEM((NC, H * E // 2, 128), u32),
            pltpu.VMEM((3 * H, NP * 8, E), u32),
            pltpu.VMEM((NC + 1, S, 128), f32),
            pltpu.VMEM((NP, 64, 128), f32),
            pltpu.VMEM((S + 8, 128), f32),
            pltpu.VMEM((2, 128, 128), f32),
            pltpu.VMEM((3, NB, 128, 128), f32),
            pltpu.VMEM((3, NB, 128, 128), f32),
            pltpu.VMEM((NB, 256, 128), f32),
            pltpu.VMEM((M, D), f32),
            pltpu.VMEM((2, H, 16, E), u32),
            pltpu.VMEM((24, H * E), u32),
            pltpu.SMEM((1,), jnp.int32),
            pltpu.VMEM((KS, D), bf16), pltpu.VMEM((D,), bf16), pltpu.VMEM((D,), bf16),
            pltpu.VMEM((M, D), bf16), pltpu.VMEM((128, 128), u32), pltpu.VMEM((64, 256), u32),
            pltpu.VMEM((NC, KS, 128), f32), pltpu.VMEM((NC, 1, 128), f32), pltpu.VMEM((1, D), f32),
            pltpu.SemaphoreType.DMA((6,)),
            pltpu.SemaphoreType.DMA((NC, 4)),
            pltpu.SemaphoreType.DMA,
            pltpu.SemaphoreType.DMA((NW,)),
            pltpu.SemaphoreType.DMA((NC,)),
            pltpu.SemaphoreType.DMA,
        ],
        compiler_params=pltpu.CompilerParams(vmem_limit_bytes=126 * 1024 * 1024),
    )(
        A_q.reshape(NP, 64, D), A_k.reshape(S, D), A_v.reshape(S, D), A_ssm_k,
        B_Wq.reshape(D // 2, 2, H, E), B_Wk.reshape(D // 2, 2, H, E), B_Wv.reshape(D // 2, 2, H, E),
        B_Wo.reshape(H * E, D),
        A_shift_k.T, A_ssm_D, gate_w, B_mem0.reshape(M, D), jnp.asarray(fwd), jnp.asarray(inv),
    )
    return out.reshape(1, S, D)
```

```python
import functools

import jax
import jax.numpy as jnp
import numpy as np
from jax import lax
import jax.experimental.pallas as pl
import jax.experimental.pallas.tpu as pltpu

f32, bf16, u32 = jnp.float32, jnp.bfloat16, jnp.uint32

S, D, H, E, M, SEG, KS = 2048, 1024, 32, 128, 8, 32, 4
NP = S // (2 * SEG)
NC = D // 128
NB = S // 128
NW = 3 * H // 2
SCALE = float(E) ** -0.5
NEG = -1000000000.0
D1, D2, HB = 2, 2, 5
KSPLIT = 2
UN = 2
MB = 64


def _unit(which, h):
    pj = h // 2
    if which == 0:
        slot = pj if pj < 8 else 8 + 5 * (pj - 8)
    else:
        slot = 8 + 5 * (pj // 2) + (1 if which == 1 else 3) + pj % 2
    return 2 * slot + h % 2


def _pack_rows(a):
    b = np.asarray(a, np.float32).astype(jnp.bfloat16).view(np.uint16).astype(np.uint32)
    return b[0::2] | (b[1::2] << 16)


def _dft_consts():
    t = np.arange(128, dtype=np.float64)
    f = np.arange(128, dtype=np.float64) + 0.5
    phi = 2.0 * np.pi * f / 256.0
    tu = np.outer(phi, t)
    tk = np.outer(phi, t - 63.5)
    ti = np.outer(np.arange(64) + 0.5, phi)
    fwd = np.concatenate([np.cos(tu), -np.sin(tu), np.cos(tk), -np.sin(tk)], axis=0)
    inv = np.concatenate([np.cos(ti), np.sin(ti)], axis=0) / 128.0
    return _pack_rows(fwd), _pack_rows(inv)


def _b(x):
    return pltpu.bitcast(x, bf16)


def _u(x):
    return pltpu.bitcast(x, u32)


def _dot(a, b):
    return jnp.dot(a, b, preferred_element_type=f32)


def _dot_t(a, b):
    return lax.dot_general(a, b, (((1,), (1,)), ((), ())), preferred_element_type=f32)


def _cat(lists):
    return [f for lst in lists for f in lst]


def _interleave(*lists):
    items = []
    for li, lst in enumerate(lists):
        for i, fn in enumerate(lst):
            items.append(((i + 0.5) / len(lst), li, i, fn))
    items.sort(key=lambda t: t[:3])
    for it in items:
        it[3]()


def _kernel(x_hbm, k_hbm, v_hbm, ssm_hbm, wq_hbm, wk_hbm, wv_hbm, wo_hbm,
            shift_hbm, ssmd_hbm, gate_hbm, mem0_hbm, fwd_hbm, inv_hbm,
            out_hbm,
            x_v, xbp, k_v, v_v, ssm_v, wraw, w_s, wo_s, bulk,
            ys, gtab, kvb, kraw, uh, kh, zz, mem_sc, kv_sc, oall, flag,
            shift_v, ssmd_v, gate_v, mem0_ref, fwd_ref, inv_ref, shift_ref, ssmd_ref, gate_ref,
            sems):
    w32 = [w.bitcast(u32) for w in (wq_hbm, wk_hbm, wv_hbm)]
    wo32 = wo_hbm.bitcast(u32)
    x32 = x_hbm.bitcast(u32)

    def kv_copies(c, sem):
        return [
            pltpu.make_async_copy(k_hbm.at[:, pl.ds(c * 128, 128)], k_v.at[c, pl.ds(16, S), :], sem),
            pltpu.make_async_copy(v_hbm.at[:, pl.ds(c * 128, 128)], v_v.at[c], sem),
        ]

    def sx_copies(c):
        return [
            pltpu.make_async_copy(ssm_hbm.at[pl.ds(c * 128, 128), :], ssm_v.at[c], sems.at[8 + c % 2]),
            pltpu.make_async_copy(x_hbm.at[pl.ds(4 * c, 4)], x_v.at[pl.ds(4 * c, 4)], sems.at[8 + c % 2]),
        ]

    def kv_next(c):
        return kv_copies(c + 1, sems.at[8 + c % 2])

    def w_copy(which, pj, slot, sem):
        return [pltpu.make_async_copy(w32[which].at[:, par, pj, :], wraw.at[slot, par], sem) for par in range(2)]

    def single_copies(t):
        return w_copy(1, 0, 9, sems.at[1]) if t == 9 else w_copy(0, t, t, sems.at[t % 8])

    def single_wait(t):
        pltpu.make_async_copy(wraw.at[t], wraw.at[t], sems.at[t % 8]).wait()

    def group_lo(g):
        sem = sems.at[2 + g % 3]
        return (w_copy(1, 2 * g + 1, 10 + 5 * g, sem) + w_copy(2, 2 * g, 11 + 5 * g, sem)
                + w_copy(2, 2 * g + 1, 12 + 5 * g, sem))

    def group_hi(g):
        sem = sems.at[2 + g % 3]
        return w_copy(0, 9 + g, 13 + 5 * g, sem) + w_copy(1, 2 * g + 2, 14 + 5 * g, sem)

    def wo_copy(j):
        return pltpu.make_async_copy(wo32.at[:, pl.ds(j * 128, 128)], wo_s.at[j], sems.at[10])

    def xb_copy():
        return pltpu.make_async_copy(x32.at[:, pl.ds(12, 8), :], xbp, sems.at[8])

    def small_copies():
        return [pltpu.make_async_copy(a, b, sems.at[10]) for a, b in
                ((shift_hbm, shift_v), (ssmd_hbm, ssmd_v), (gate_hbm, gate_v), (mem0_hbm, mem0_ref),
                 (fwd_hbm, fwd_ref), (inv_hbm, inv_ref))] + kv_copies(0, sems.at[10])

    def start_all(cps):
        for cp in cps:
            cp.start()

    def wait_all(cps):
        for cp in cps:
            cp.wait()

    def start_head_batch(t):
        start_all({0: lambda: _cat(single_copies(u) for u in range(4, 8)),
                   2: lambda: sx_copies(0) + kv_next(0) + single_copies(8) + single_copies(9),
                   4: lambda: group_lo(0) + group_hi(0),
                   6: lambda: sx_copies(1) + kv_next(1) + group_lo(1) + group_hi(1)}[t]())

    def start_late_batch(i):
        g = i + 2
        cps = sx_copies(g) + (kv_next(g) if g < NC - 1 else []) + group_lo(g) + (group_hi(g) if g < NC - 1 else [])
        if i < NC // 2:
            cps += [wo_copy(2 * i), wo_copy(2 * i + 1)]
        start_all(cps)

    def once_if(cond, fn):
        def body(_, carry):
            fn()
            return carry
        lax.fori_loop(0, cond.astype(jnp.int32), body, 0)

    start_all(single_copies(0) + [xb_copy()] + _cat(single_copies(u) for u in range(1, 4)) + small_copies())

    flag[0] = 1
    for c in range(NC):
        k_v[c, 0:16, :] = jnp.zeros((16, 128), bf16)

    def pre(c, ys_c, b, n=128):
        r0 = b * n if isinstance(b, int) else pl.multiple_of(b * n, n)
        h0 = b * (n // 2) if isinstance(b, int) else pl.multiple_of(b * (n // 2), n // 2)
        sh = shift_ref[c]
        kx = k_v[c, pl.ds(r0, n + 16), :].astype(f32)[8:]
        ks = kx[8:] * sh[0:1, :]
        for j in range(1, KS):
            ks = ks + kx[8 - j:8 + n - j] * sh[j:j + 1, :]
        kv = (ks * v_v[c, pl.ds(r0, n), :].astype(f32)).astype(bf16)
        ys_c[pl.ds(r0, n), :] = kv.astype(f32) * ssmd_ref[c]
        kvb[pl.ds(h0, n // 2), :] = _u(kv)

    def fwd_thunks(c, cn, ys_n):
        def fu(i):
            kv = _b(kvb[64 * i:64 * (i + 1), :])
            ur = _dot(_b(fwd_ref[0:64, :]), kv)
            ui = _dot(_b(fwd_ref[64:128, :]), kv)
            uh[0, i] = ur
            uh[1, i] = ui
            uh[2, i] = ur + ui

        def fk(i):
            kb = ssm_v[c, :, 128 * i:128 * (i + 1)]
            kr = _dot_t(_b(fwd_ref[128:192, :]), kb)
            ki = _dot_t(_b(fwd_ref[192:256, :]), kb)
            if i == 0:
                pr, pi = kr, ki
            else:
                row = lax.broadcasted_iota(jnp.int32, (128, 128), 0)
                sgn = jnp.where(row % 2 == 0, 1.0, -1.0).astype(f32)
                pr = kr - sgn * kraw[1]
                pi = ki + sgn * kraw[0]
            kraw[0] = kr
            kraw[1] = ki
            kh[0, i] = pr
            kh[1, i] = pi
            kh[2, i] = pr + pi

        return _cat([functools.partial(fu, i), functools.partial(fk, i), functools.partial(pre, cn, ys_n, i)]
                    for i in range(NB))

    def group4(comp, rows, b):
        acc = None
        for j in range(4 * b + 4):
            lo = max(0, j - 4 * b)
            t = kh[comp, 4 * b + lo - j:4 * b + 4 - j, rows, :] * uh[comp, j, rows, :][None]
            if acc is None:
                acc = t
            elif lo == 0:
                acc = acc + t
            else:
                acc = jnp.concatenate([acc[:lo], acc[lo:] + t], axis=0)
        return acc

    def mac_thunks(p):
        rows, rows2 = pl.ds(8 * p, 8), pl.ds(128 + 8 * p, 8)
        out = []
        for b in range(4):
            st = {}

            def f0(b=b, st=st):
                st['a'] = group4(0, rows, b)

            def f1(b=b, st=st):
                bb = group4(1, rows, b)
                a = st.pop('a')
                zz[4 * b:4 * b + 4, rows, :] = a - bb
                st['ab'] = a + bb

            def f2(b=b, st=st):
                zz[4 * b:4 * b + 4, rows2, :] = group4(2, rows, b) - st.pop('ab')

            out += [f0, f1, f2]
        return out

    def inv_thunks(ys_c):
        def f(i):
            a = _dot(_b(inv_ref[0:32, :]), zz[i, 0:128, :].astype(bf16))
            b = _dot(_b(inv_ref[32:64, :]), zz[i, 128:256, :].astype(bf16))
            lo = a + b
            rev = 7 - lax.broadcasted_iota(jnp.int32, (8, 128), 0)
            y = jnp.concatenate(
                [jnp.take_along_axis(lo[8 * r:8 * r + 8], rev, axis=0) for r in range(7, -1, -1)] + [a - b],
                axis=0)
            ys_c[128 * i:128 * (i + 1), :] = ys_c[128 * i:128 * (i + 1), :] + y.astype(bf16).astype(f32)
        return [functools.partial(f, i) for i in range(NB)]

    def gate_thunks(i):
        def f(r):
            rows = pl.ds(32 * (r % 2), 32)
            xo = x_v[4 * i + r // 2, rows, :].astype(f32)
            g = jax.nn.sigmoid(jnp.sum(xo * gate_ref[...], axis=-1, keepdims=True))
            gtab[4 * i + r // 2, rows, :] = jnp.broadcast_to(g, (32, 128))
        return [functools.partial(f, r) for r in range(8)]

    def repack_thunks(src, dst):
        def f(db):
            r = pl.ds(db * 64, 64)
            ev, od = src[0, r, :], src[1, r, :]
            dst[0, r, :] = (ev & jnp.uint32(0xFFFF)) | (od << 16)
            dst[1, r, :] = (ev >> 16) | (od & jnp.uint32(0xFFFF0000))
        return [functools.partial(f, db) for db in range(8)]

    def bulk_thunks(wsrc, dst, nk=1):
        st = {}

        def f(mc, kk):
            kw = D // nk
            lhs = xbp[mc * (MB // 16):(mc + 1) * (MB // 16), :, kk * kw:(kk + 1) * kw].reshape(MB // 2, kw)
            r = _dot(_b(lhs), _b(wsrc[kk * kw // 2:(kk + 1) * kw // 2, :]))
            if kk > 0:
                r = r + st.pop(mc)
            if kk < nk - 1:
                st[mc] = r
            else:
                dst[mc * (MB // 2):(mc + 1) * (MB // 2), :] = _u(r.astype(bf16))
        return [functools.partial(f, mc, kk) for mc in range(NP * 16 // MB) for kk in range(nk)]

    single_wait(0)
    _interleave(repack_thunks(wraw.at[0], w_s.at[pl.ds(0, 2)]))
    xb_copy().wait()

    start_head_batch(0)

    @pl.when(flag[0] > 0)
    def _():
        _interleave(_cat(bulk_thunks(w_s.at[u], bulk.at[u]) for u in range(2)))

    single_wait(1)
    _interleave(repack_thunks(wraw.at[1], w_s.at[pl.ds(2, 2)]))

    def head(with_pre, t, carry):
        for c in ((4, 6) if with_pre else (2,)):
            once_if(t == c, functools.partial(start_head_batch, c))
        single_wait(t + 1)
        wwin = w_s.at[pl.ds(t * 2, 4)]
        bwin = bulk.at[pl.ds(t * 2, 2)]

        @pl.when(flag[0] > 0)
        def _():
            lists = [_cat(bulk_thunks(wwin.at[u], bwin.at[u]) for u in range(2)),
                     repack_thunks(wraw.at[t + 1], wwin.at[pl.ds(2, 2)])]
            if with_pre:
                lists.append([functools.partial(pre, 0, ys.at[0], 8 * (t - 4) + b, 64) for b in range(8)])
            _interleave(*lists)
        return carry

    lax.fori_loop(1, 4, functools.partial(head, False), 0)
    wait_all(small_copies())
    sh32 = shift_v[...].astype(f32)
    sd32 = ssmd_v[...].reshape(1, D).astype(f32)
    for c in range(NC):
        shift_ref[c] = sh32[:, c * 128:(c + 1) * 128]
        ssmd_ref[c] = sd32[:, c * 128:(c + 1) * 128]
    gate_ref[...] = gate_v[...].reshape(1, D).astype(f32)
    lax.fori_loop(4, 8, functools.partial(head, True), 0)
    single_wait(9)
    _interleave(repack_thunks(wraw.at[9], w_s.at[pl.ds(18, 2)]))
    wait_all(sx_copies(0) + kv_next(0))

    def block_b(i):
        first = isinstance(i, int)
        wwin = w_s.at[pl.ds(16 + i * 10, 2)]
        bwin = bulk.at[pl.ds(16 + i * 10, 2)]
        ywin = ys.at[pl.ds(0 if first else i - 1, 3)]
        lists = [_cat(bulk_thunks(wwin.at[u], bwin.at[u]) for u in range(2)),
                 fwd_thunks(i, 1 if first else jnp.minimum(i + 1, NC - 1), ywin.at[1 if first else 2]),
                 gate_thunks(i)]
        if not first:
            lists.insert(2, inv_thunks(ywin.at[0]))
        _interleave(*lists)

    @pl.when(flag[0] > 0)
    def _():
        block_b(0)

    def pro(i, carry):
        wwin = w_s.at[pl.ds(18 + i * 10, 12)]
        bwin = bulk.at[pl.ds(18 + i * 10, 8)]
        rwin = wraw.at[pl.ds(10 + i * 5, 5)]
        gsem = sems.at[2 + i % 3]
        pltpu.make_async_copy(rwin.at[0:3], rwin.at[0:3], gsem).wait()

        @pl.when(i < NC - 1)
        def _():
            pltpu.make_async_copy(rwin.at[3:5], rwin.at[3:5], gsem).wait()

        for c in range(NC - 2):
            once_if(i == c, functools.partial(start_late_batch, c))

        @pl.when(flag[0] > 0)
        def _():
            _interleave(_cat(bulk_thunks(wwin.at[u], bwin.at[u], 2) for u in range(8)),
                        _cat(mac_thunks(p) for p in range(16)),
                        _cat(repack_thunks(rwin.at[t], wwin.at[pl.ds(2 + 2 * t, 2)]) for t in range(5)))

        @pl.when(i < NC - 1)
        def _():
            wait_all(sx_copies(jnp.minimum(i + 1, NC - 1)))

        @pl.when(i < NC - 2)
        def _():
            wait_all(kv_next(jnp.minimum(i + 1, NC - 2)))

        @pl.when(i < NC - 1)
        def _():
            block_b(jnp.minimum(i + 1, NC - 1))
        return carry

    lax.fori_loop(0, NC, pro, 0)
    _interleave(inv_thunks(ys.at[NC - 1]))
    wait_all([wo_copy(j) for j in range(NC)])

    mem_sc[...] = mem0_ref[...].astype(f32)

    ra = lax.broadcasted_iota(jnp.int32, (32, 48), 0)
    ca = lax.broadcasted_iota(jnp.int32, (32, 48), 1)
    same_a = ca < 40
    mask_a = same_a & ((ra < M) | (ra >= ca))
    rb = lax.broadcasted_iota(jnp.int32, (48, 80), 0)
    cb = lax.broadcasted_iota(jnp.int32, (48, 80), 1)
    q_in_a = (rb >= 32) & (rb < 40)
    k_in_a = ((cb >= 32) & (cb < 40)) | (cb >= 48)
    qpos = jnp.where(rb < 8, rb, jnp.where(rb < 32, rb + 8, jnp.where(rb < 40, rb, rb - 32)))
    kpos = jnp.where(cb < 8, cb, jnp.where(cb < 32, cb + 8,
                     jnp.where(cb < 40, cb, jnp.where(cb < 48, cb - 32, cb - 48))))
    same_b = q_in_a == k_in_a
    mask_b = same_b & ((qpos < M) | (qpos >= kpos))
    fill_a = jnp.where(same_a, NEG, -jnp.inf).astype(f32)
    fill_b = jnp.where(same_b, NEG, -jnp.inf).astype(f32)

    def step(first, jp, side):
        xr = x_v[jp, 0:24, :] if first else x_v[jp, 40:64, :]
        lhs = jnp.concatenate([mem_sc[...], xr.astype(f32)], axis=0).astype(bf16)
        nw = 32 if first else 48
        mask, fill = (mask_a, fill_a) if first else (mask_b, fill_b)
        br = pl.ds(pl.multiple_of(jp * 8, 8), 8)
        qkv, ps, part = {}, {}, {}

        def proj_lo(h):
            part[h] = [_dot(lhs[:, :D // 2], _b(w_s[_unit(t, h), 0:D // 4, :])) for t in range(3)]

        def proj(h):
            if h in part:
                low = part.pop(h)
                q, k, v = [(_dot(lhs[:, D // 2:], _b(w_s[_unit(t, h), D // 4:, :])) + low[t]).astype(bf16)
                           for t in range(3)]
            else:
                q, k, v = [_dot(lhs, _b(w_s[_unit(t, h)])).astype(bf16) for t in range(3)]
            kb = _b(bulk[_unit(1, h), br, :])
            vb = _b(bulk[_unit(2, h), br, :])
            if first:
                kv_sc[0, h] = _u(k)
                kv_sc[1, h] = _u(v)
                k = jnp.concatenate([k, kb], axis=0)
                v = jnp.concatenate([v, vb], axis=0)
            else:
                q = jnp.concatenate([q, _b(bulk[_unit(0, h), br, :])], axis=0)
                k = jnp.concatenate([k, kb, _b(kv_sc[0, h])], axis=0)
                v = jnp.concatenate([v, vb, _b(kv_sc[1, h])], axis=0)
            qkv[h] = (q, k, v)

        def qk(h):
            q, k, _ = qkv[h]
            s = jnp.where(mask, _dot_t(q, k) * SCALE, fill)
            p = jnp.exp(s - jnp.max(s, axis=-1, keepdims=True))
            den = jnp.sum(p, axis=-1, keepdims=True)
            ps[h] = (p * pl.reciprocal(den, approx=False)).astype(bf16)

        def pv(h):
            o = _dot(ps.pop(h), qkv.pop(h)[2])
            oall[0:nw // 2, h * 128:(h + 1) * 128] = _u(o.astype(bf16))

        side = list(side)
        for h in range(KSPLIT):
            proj_lo(h)
        for h in range(H):
            proj(h)
            if h - D1 >= 0:
                qk(h - D1)
            if h - D1 - D2 >= 0:
                pv(h - D1 - D2)
            if side and h >= 4 and h % 2 == 0:
                side.pop(0)()

        ka = (H - HB) * 128
        oa = _b(oall[0:nw // 2, 0:ka])
        accs = []
        nslot = D1 + D2 + 1
        for i in range(nslot):
            while len(accs) < (NC * (i + 1)) // nslot:
                accs.append(_dot(oa, _b(wo_s[len(accs), 0:ka // 2, :])))
            if i < D1:
                qk(H + i - D1)
            if i < D1 + D2:
                pv(H + i - D1 - D2)
        ob = _b(oall[0:nw // 2, ka:])
        res = [_dot(ob, _b(wo_s[j, ka // 2:, :])) + accs[j] for j in range(NC)]

        mem_sc[...] = jnp.concatenate([r[:M] for r in res], axis=1).astype(bf16).astype(f32)

        lo, n = (0, 24) if first else (24, 40)

        def mix(j):
            if first:
                bj = res[j][8:32]
            else:
                bj = jnp.concatenate([res[j][32:48], res[j][8:32]], axis=0)
            cols = slice(j * 128, (j + 1) * 128)
            aj = x_v[jp, lo:lo + n, cols].astype(f32) * ys[j, pl.ds(pl.multiple_of(jp * 64 + lo, 8), n), :]
            x_v[jp, lo:lo + n, cols] = (bj + gtab[jp, lo:lo + n, :] * (aj - bj)).astype(bf16)

        return [functools.partial(mix, j) for j in range(NC)]

    def pairs(jq, carry):
        epi = []
        for r in range(UN):
            for first in (True, False):
                epi = step(first, jq * UN + r, epi)
        _interleave(epi)
        rows = pl.ds(jq * UN, UN)
        pltpu.make_async_copy(x_v.at[rows], out_hbm.at[rows], sems.at[10]).start()
        return carry

    lax.fori_loop(0, NP // UN, pairs, 0)
    pltpu.make_async_copy(x_v, out_hbm, sems.at[10]).wait()


@functools.partial(jax.jit, static_argnames=("B_seg_len",))
def pallas_gated_mix__ssm_conv_h3__memory_aug_recurrent_mem_tr__prompt_kernel(
    A_q, A_k, A_v, A_shift_k, A_ssm_k, A_ssm_D, B_x, B_mem0, B_Wq, B_Wk, B_Wv, B_Wo,
    B_seg_len, gate_w,
):
    del B_x
    assert int(B_seg_len) == SEG and A_q.shape == (1, S, D) and B_Wq.shape == (D, H, E)
    fwd, inv = _dft_consts()
    out = pl.pallas_call(
        _kernel,
        out_shape=jax.ShapeDtypeStruct((NP, 64, D), bf16),
        in_specs=[pl.BlockSpec(memory_space=pl.ANY)] * 14,
        out_specs=pl.BlockSpec(memory_space=pl.ANY),
        scratch_shapes=[
            pltpu.VMEM((NP, 64, D), bf16),
            pltpu.VMEM((NP, 8, D), u32),
            pltpu.VMEM((NC, S + 64, 128), bf16),
            pltpu.VMEM((NC, S, 128), bf16),
            pltpu.VMEM((NC, 128, S), bf16),
            pltpu.VMEM((NW + 2, 2, D // 2, E), u32),
            pltpu.VMEM((3 * H + 4, D // 2, E), u32),
            pltpu.VMEM((NC, H * E // 2, 128), u32),
            pltpu.VMEM((3 * H, NP * 8, E), u32),
            pltpu.VMEM((NC + 1, S, 128), f32),
            pltpu.VMEM((NP, 64, 128), f32),
            pltpu.VMEM((S // 2, 128), u32),
            pltpu.VMEM((2, 128, 128), f32),
            pltpu.VMEM((3, NB, 128, 128), f32),
            pltpu.VMEM((3, NB, 128, 128), f32),
            pltpu.VMEM((NB, 256, 128), f32),
            pltpu.VMEM((M, D), f32),
            pltpu.VMEM((2, H, 16, E), u32),
            pltpu.VMEM((24, H * E), u32),
            pltpu.SMEM((1,), jnp.int32),
            pltpu.VMEM((KS, D), bf16), pltpu.VMEM((D,), bf16), pltpu.VMEM((D,), bf16),
            pltpu.VMEM((M, D), bf16), pltpu.VMEM((256, 128), u32), pltpu.VMEM((64, 128), u32),
            pltpu.VMEM((NC, KS, 128), f32), pltpu.VMEM((NC, 1, 128), f32), pltpu.VMEM((1, D), f32),
            pltpu.SemaphoreType.DMA((11,)),
        ],
        compiler_params=pltpu.CompilerParams(vmem_limit_bytes=126 * 1024 * 1024),
    )(
        A_q.reshape(NP, 64, D), A_k.reshape(S, D), A_v.reshape(S, D), A_ssm_k,
        B_Wq.reshape(D // 2, 2, H, E), B_Wk.reshape(D // 2, 2, H, E), B_Wv.reshape(D // 2, 2, H, E),
        B_Wo.reshape(H * E, D),
        A_shift_k.T, A_ssm_D, gate_w, B_mem0.reshape(M, D), jnp.asarray(fwd), jnp.asarray(inv),
    )
    return out.reshape(1, S, D)
```

```python
import functools

import jax
import jax.numpy as jnp
import numpy as np
from jax import lax
import jax.experimental.pallas as pl
import jax.experimental.pallas.tpu as pltpu

f32, bf16, u32 = jnp.float32, jnp.bfloat16, jnp.uint32

S, D, H, E, M, SEG, KS = 2048, 1024, 32, 128, 8, 32, 4
NP = S // (2 * SEG)
NC = D // 128
NB = S // 128
NW = 3 * H // 2
SCALE = float(E) ** -0.5
NEG = -1000000000.0
D1, D2, HB = 2, 2, 5
KSPLIT = 2
UN = 2
MB = 64


def _unit(which, h):
    pj = h // 2
    if which == 0:
        slot = pj if pj < 8 else 8 + 5 * (pj - 8)
    else:
        slot = 8 + 5 * (pj // 2) + (1 if which == 1 else 3) + pj % 2
    return 2 * slot + h % 2


def _pack_rows(a):
    b = np.asarray(a, np.float32).astype(jnp.bfloat16).view(np.uint16).astype(np.uint32)
    return b[0::2] | (b[1::2] << 16)


def _dft_consts():
    t = np.arange(128, dtype=np.float64)
    f = np.arange(128, dtype=np.float64) + 0.5
    phi = 2.0 * np.pi * f / 256.0
    tu = np.outer(phi, t)
    tk = np.outer(phi, t - 63.5)
    ti = np.outer(np.arange(64) + 0.5, phi)
    fwd = np.concatenate([np.cos(tu), -np.sin(tu), np.cos(tk), -np.sin(tk)], axis=0)
    inv = np.concatenate([np.cos(ti), np.sin(ti)], axis=0) / 128.0
    return _pack_rows(fwd), _pack_rows(inv)


def _b(x):
    return pltpu.bitcast(x, bf16)


def _u(x):
    return pltpu.bitcast(x, u32)


def _dot(a, b):
    return jnp.dot(a, b, preferred_element_type=f32)


def _dot_t(a, b):
    return lax.dot_general(a, b, (((1,), (1,)), ((), ())), preferred_element_type=f32)


def _cat(lists):
    return [f for lst in lists for f in lst]


def _interleave(*lists):
    items = []
    for li, lst in enumerate(lists):
        for i, fn in enumerate(lst):
            items.append(((i + 0.5) / len(lst), li, i, fn))
    items.sort(key=lambda t: t[:3])
    for it in items:
        it[3]()


def _kernel(x_hbm, k_hbm, v_hbm, ssm_hbm, wq_hbm, wk_hbm, wv_hbm, wo_hbm,
            shift_hbm, ssmd_hbm, gate_hbm, mem0_hbm, fwd_hbm, inv_hbm,
            out_hbm,
            x_v, xbp, k_v, v_v, ssm_v, wraw, w_s, wo_s, bulk,
            ys, gtab, kvb, kraw, uh, kh, zz, mem_sc, kv_sc, oall, flag,
            shift_v, ssmd_v, gate_v, mem0_ref, fwd_ref, inv_ref, shift_ref, ssmd_ref, gate_ref,
            sems):
    w32 = [w.bitcast(u32) for w in (wq_hbm, wk_hbm, wv_hbm)]
    wo32 = wo_hbm.bitcast(u32)
    x32 = x_hbm.bitcast(u32)

    def kv_copies(c, sem):
        return [
            pltpu.make_async_copy(k_hbm.at[:, pl.ds(c * 128, 128)], k_v.at[c, pl.ds(16, S), :], sem),
            pltpu.make_async_copy(v_hbm.at[:, pl.ds(c * 128, 128)], v_v.at[c], sem),
        ]

    def sx_copies(c):
        return [
            pltpu.make_async_copy(ssm_hbm.at[pl.ds(c * 128, 128), :], ssm_v.at[c], sems.at[8 + c % 2]),
            pltpu.make_async_copy(x_hbm.at[pl.ds(4 * c, 4)], x_v.at[pl.ds(4 * c, 4)], sems.at[8 + c % 2]),
        ]

    def kv_next(c):
        return kv_copies(c + 1, sems.at[8 + c % 2])

    def w_copy(which, pj, slot, sem):
        return [pltpu.make_async_copy(w32[which].at[:, par, pj, :], wraw.at[slot, par], sem) for par in range(2)]

    def single_copies(t):
        return w_copy(1, 0, 9, sems.at[1]) if t == 9 else w_copy(0, t, t, sems.at[t % 8])

    def single_wait(t):
        pltpu.make_async_copy(wraw.at[t], wraw.at[t], sems.at[t % 8]).wait()

    def group_lo(g):
        sem = sems.at[2 + g % 3]
        return (w_copy(1, 2 * g + 1, 10 + 5 * g, sem) + w_copy(2, 2 * g, 11 + 5 * g, sem)
                + w_copy(2, 2 * g + 1, 12 + 5 * g, sem))

    def group_hi(g):
        sem = sems.at[2 + g % 3]
        return w_copy(0, 9 + g, 13 + 5 * g, sem) + w_copy(1, 2 * g + 2, 14 + 5 * g, sem)

    def wo_copy(j):
        return pltpu.make_async_copy(wo32.at[:, pl.ds(j * 128, 128)], wo_s.at[j], sems.at[10])

    def xb_copy():
        return pltpu.make_async_copy(x32.at[:, pl.ds(12, 8), :], xbp, sems.at[8])

    def small_copies():
        return [pltpu.make_async_copy(a, b, sems.at[10]) for a, b in
                ((shift_hbm, shift_v), (ssmd_hbm, ssmd_v), (gate_hbm, gate_v), (mem0_hbm, mem0_ref),
                 (fwd_hbm, fwd_ref), (inv_hbm, inv_ref))] + kv_copies(0, sems.at[10])

    def start_all(cps):
        for cp in cps:
            cp.start()

    def wait_all(cps):
        for cp in cps:
            cp.wait()

    def start_head_batch(t):
        start_all({0: lambda: _cat(single_copies(u) for u in range(4, 8)),
                   2: lambda: sx_copies(0) + kv_next(0) + single_copies(8) + single_copies(9),
                   4: lambda: group_lo(0) + group_hi(0),
                   6: lambda: sx_copies(1) + kv_next(1) + group_lo(1) + group_hi(1)}[t]())

    def start_late_batch(i):
        g = i + 2
        cps = sx_copies(g) + (kv_next(g) if g < NC - 1 else []) + group_lo(g) + (group_hi(g) if g < NC - 1 else [])
        if i < NC // 2:
            cps += [wo_copy(2 * i), wo_copy(2 * i + 1)]
        start_all(cps)

    def once_if(cond, fn):
        def body(_, carry):
            fn()
            return carry
        lax.fori_loop(0, cond.astype(jnp.int32), body, 0)

    start_all(single_copies(0) + [xb_copy()] + _cat(single_copies(u) for u in range(1, 4)) + small_copies())

    flag[0] = 1
    for c in range(NC):
        k_v[c, 0:16, :] = jnp.zeros((16, 128), bf16)

    ra = lax.broadcasted_iota(jnp.int32, (32, 48), 0)
    ca = lax.broadcasted_iota(jnp.int32, (32, 48), 1)
    same_a = ca < 40
    mask_a = same_a & ((ra < M) | (ra >= ca))
    rb = lax.broadcasted_iota(jnp.int32, (48, 80), 0)
    cb = lax.broadcasted_iota(jnp.int32, (48, 80), 1)
    q_in_a = (rb >= 32) & (rb < 40)
    k_in_a = ((cb >= 32) & (cb < 40)) | (cb >= 48)
    qpos = jnp.where(rb < 8, rb, jnp.where(rb < 32, rb + 8, jnp.where(rb < 40, rb, rb - 32)))
    kpos = jnp.where(cb < 8, cb, jnp.where(cb < 32, cb + 8,
                     jnp.where(cb < 40, cb, jnp.where(cb < 48, cb - 32, cb - 48))))
    same_b = q_in_a == k_in_a
    mask_b = same_b & ((qpos < M) | (qpos >= kpos))
    fill_a = jnp.where(same_a, NEG, -jnp.inf).astype(f32)
    fill_b = jnp.where(same_b, NEG, -jnp.inf).astype(f32)

    def pre(c, ys_c, b, n=128):
        r0 = b * n if isinstance(b, int) else pl.multiple_of(b * n, n)
        h0 = b * (n // 2) if isinstance(b, int) else pl.multiple_of(b * (n // 2), n // 2)
        sh = shift_ref[c]
        kx = k_v[c, pl.ds(r0, n + 16), :].astype(f32)[8:]
        ks = kx[8:] * sh[0:1, :]
        for j in range(1, KS):
            ks = ks + kx[8 - j:8 + n - j] * sh[j:j + 1, :]
        kv = (ks * v_v[c, pl.ds(r0, n), :].astype(f32)).astype(bf16)
        ys_c[pl.ds(r0, n), :] = kv.astype(f32) * ssmd_ref[c]
        kvb[pl.ds(h0, n // 2), :] = _u(kv)

    def fwd_thunks(c, cn, ys_n):
        def fu(i):
            kv = _b(kvb[64 * i:64 * (i + 1), :])
            ur = _dot(_b(fwd_ref[0:64, :]), kv)
            ui = _dot(_b(fwd_ref[64:128, :]), kv)
            uh[0, i] = ur
            uh[1, i] = ui
            uh[2, i] = ur + ui

        def fk(i):
            kb = ssm_v[c, :, 128 * i:128 * (i + 1)]
            kr = _dot_t(_b(fwd_ref[128:192, :]), kb)
            ki = _dot_t(_b(fwd_ref[192:256, :]), kb)
            if i == 0:
                pr, pi = kr, ki
            else:
                row = lax.broadcasted_iota(jnp.int32, (128, 128), 0)
                sgn = jnp.where(row % 2 == 0, 1.0, -1.0).astype(f32)
                pr = kr - sgn * kraw[1]
                pi = ki + sgn * kraw[0]
            kraw[0] = kr
            kraw[1] = ki
            kh[0, i] = pr
            kh[1, i] = pi
            kh[2, i] = pr + pi

        return _cat([functools.partial(fu, i), functools.partial(fk, i), functools.partial(pre, cn, ys_n, i)]
                    for i in range(NB))

    def group4(comp, rows, b):
        acc = None
        for j in range(4 * b + 4):
            lo = max(0, j - 4 * b)
            t = kh[comp, 4 * b + lo - j:4 * b + 4 - j, rows, :] * uh[comp, j, rows, :][None]
            if acc is None:
                acc = t
            elif lo == 0:
                acc = acc + t
            else:
                acc = jnp.concatenate([acc[:lo], acc[lo:] + t], axis=0)
        return acc

    def mac_thunks(p):
        rows, rows2 = pl.ds(8 * p, 8), pl.ds(128 + 8 * p, 8)
        out = []
        for b in range(4):
            st = {}

            def f0(b=b, st=st):
                st['a'] = group4(0, rows, b)

            def f1(b=b, st=st):
                bb = group4(1, rows, b)
                a = st.pop('a')
                zz[4 * b:4 * b + 4, rows, :] = a - bb
                st['ab'] = a + bb

            def f2(b=b, st=st):
                zz[4 * b:4 * b + 4, rows2, :] = group4(2, rows, b) - st.pop('ab')

            out += [f0, f1, f2]
        return out

    def inv_thunks(ys_c):
        def f(i):
            a = _dot(_b(inv_ref[0:32, :]), zz[i, 0:128, :].astype(bf16))
            b = _dot(_b(inv_ref[32:64, :]), zz[i, 128:256, :].astype(bf16))
            lo = a + b
            rev = 7 - lax.broadcasted_iota(jnp.int32, (8, 128), 0)
            y = jnp.concatenate(
                [jnp.take_along_axis(lo[8 * r:8 * r + 8], rev, axis=0) for r in range(7, -1, -1)] + [a - b],
                axis=0)
            ys_c[128 * i:128 * (i + 1), :] = ys_c[128 * i:128 * (i + 1), :] + y.astype(bf16).astype(f32)
        return [functools.partial(f, i) for i in range(NB)]

    def gate_thunks(i):
        def f(r):
            rows = pl.ds(32 * (r % 2), 32)
            xo = x_v[4 * i + r // 2, rows, :].astype(f32)
            g = jax.nn.sigmoid(jnp.sum(xo * gate_ref[...], axis=-1, keepdims=True))
            gtab[4 * i + r // 2, rows, :] = jnp.broadcast_to(g, (32, 128))
        return [functools.partial(f, r) for r in range(8)]

    def repack_thunks(src, dst):
        def f(db):
            r = pl.ds(db * 64, 64)
            ev, od = src[0, r, :], src[1, r, :]
            dst[0, r, :] = (ev & jnp.uint32(0xFFFF)) | (od << 16)
            dst[1, r, :] = (ev >> 16) | (od & jnp.uint32(0xFFFF0000))
        return [functools.partial(f, db) for db in range(8)]

    def bulk_thunks(wsrc, dst, nk=1):
        st = {}

        def f(mc, kk):
            kw = D // nk
            lhs = xbp[mc * (MB // 16):(mc + 1) * (MB // 16), :, kk * kw:(kk + 1) * kw].reshape(MB // 2, kw)
            r = _dot(_b(lhs), _b(wsrc[kk * kw // 2:(kk + 1) * kw // 2, :]))
            if kk > 0:
                r = r + st.pop(mc)
            if kk < nk - 1:
                st[mc] = r
            else:
                dst[mc * (MB // 2):(mc + 1) * (MB // 2), :] = _u(r.astype(bf16))
        return [functools.partial(f, mc, kk) for mc in range(NP * 16 // MB) for kk in range(nk)]

    single_wait(0)
    _interleave(repack_thunks(wraw.at[0], w_s.at[pl.ds(0, 2)]))
    xb_copy().wait()

    start_head_batch(0)

    @pl.when(flag[0] > 0)
    def _():
        _interleave(_cat(bulk_thunks(w_s.at[u], bulk.at[u]) for u in range(2)))

    single_wait(1)
    _interleave(repack_thunks(wraw.at[1], w_s.at[pl.ds(2, 2)]))

    def head(with_pre, t, carry):
        for c in ((4,) if with_pre else (2,)):
            once_if(t == c, functools.partial(start_head_batch, c))
        single_wait(t + 1)
        wwin = w_s.at[pl.ds(t * 2, 4)]
        bwin = bulk.at[pl.ds(t * 2, 2)]

        @pl.when(flag[0] > 0)
        def _():
            lists = [_cat(bulk_thunks(wwin.at[u], bwin.at[u]) for u in range(2)),
                     repack_thunks(wraw.at[t + 1], wwin.at[pl.ds(2, 2)])]
            if with_pre:
                lists.append([functools.partial(pre, 0, ys.at[0], 8 * (t - 4) + b, 64) for b in range(8)])
            _interleave(*lists)
        return carry

    lax.fori_loop(1, 4, functools.partial(head, False), 0)
    wait_all(small_copies())
    sh32 = shift_v[...].astype(f32)
    sd32 = ssmd_v[...].reshape(1, D).astype(f32)
    for c in range(NC):
        shift_ref[c] = sh32[:, c * 128:(c + 1) * 128]
        ssmd_ref[c] = sd32[:, c * 128:(c + 1) * 128]
    gate_ref[...] = gate_v[...].reshape(1, D).astype(f32)
    mem_sc[...] = mem0_ref[...].astype(f32)
    lax.fori_loop(4, 8, functools.partial(head, True), 0)
    single_wait(9)
    _interleave(repack_thunks(wraw.at[9], w_s.at[pl.ds(18, 2)]))
    wait_all(sx_copies(0) + kv_next(0))
    start_head_batch(6)

    def block_b(i):
        first = isinstance(i, int)
        wwin = w_s.at[pl.ds(16 + i * 10, 2)]
        bwin = bulk.at[pl.ds(16 + i * 10, 2)]
        ywin = ys.at[pl.ds(0 if first else i - 1, 3)]
        lists = [_cat(bulk_thunks(wwin.at[u], bwin.at[u]) for u in range(2)),
                 fwd_thunks(i, 1 if first else jnp.minimum(i + 1, NC - 1), ywin.at[1 if first else 2]),
                 gate_thunks(i)]
        if not first:
            lists.insert(2, inv_thunks(ywin.at[0]))
        _interleave(*lists)

    @pl.when(flag[0] > 0)
    def _():
        block_b(0)

    def pro(i, carry):
        wwin = w_s.at[pl.ds(18 + i * 10, 12)]
        bwin = bulk.at[pl.ds(18 + i * 10, 8)]
        rwin = wraw.at[pl.ds(10 + i * 5, 5)]
        gsem = sems.at[2 + i % 3]

        @pl.when(i < NC - 1)
        def _():
            pltpu.make_async_copy(rwin, rwin, gsem).wait()

        @pl.when(i == NC - 1)
        def _():
            pltpu.make_async_copy(rwin.at[0:3], rwin.at[0:3], gsem).wait()

        for c in range(NC - 2):
            once_if(i == c, functools.partial(start_late_batch, c))

        @pl.when(flag[0] > 0)
        def _():
            _interleave(_cat(bulk_thunks(wwin.at[u], bwin.at[u], 2) for u in range(8)),
                        _cat(mac_thunks(p) for p in range(16)),
                        _cat(repack_thunks(rwin.at[t], wwin.at[pl.ds(2 + 2 * t, 2)]) for t in range(5)))

        @pl.when(i < NC - 1)
        def _():
            wait_all(sx_copies(jnp.minimum(i + 1, NC - 1)))

        @pl.when(i < NC - 2)
        def _():
            wait_all(kv_next(jnp.minimum(i + 1, NC - 2)))

        @pl.when(i < NC - 1)
        def _():
            block_b(jnp.minimum(i + 1, NC - 1))
        return carry

    lax.fori_loop(0, NC, pro, 0)
    _interleave(inv_thunks(ys.at[NC - 1]))
    wait_all([wo_copy(j) for j in range(NC)])

    def step(first, jp, side):
        xr = x_v[jp, 0:24, :] if first else x_v[jp, 40:64, :]
        lhs = jnp.concatenate([mem_sc[...], xr.astype(f32)], axis=0).astype(bf16)
        nw = 32 if first else 48
        mask, fill = (mask_a, fill_a) if first else (mask_b, fill_b)
        br = pl.ds(pl.multiple_of(jp * 8, 8), 8)
        qkv, ps, part = {}, {}, {}

        def proj_lo(h):
            part[h] = [_dot(lhs[:, :D // 2], _b(w_s[_unit(t, h), 0:D // 4, :])) for t in range(3)]

        def proj(h):
            if h in part:
                low = part.pop(h)
                q, k, v = [(_dot(lhs[:, D // 2:], _b(w_s[_unit(t, h), D // 4:, :])) + low[t]).astype(bf16)
                           for t in range(3)]
            else:
                q, k, v = [_dot(lhs, _b(w_s[_unit(t, h)])).astype(bf16) for t in range(3)]
            kb = _b(bulk[_unit(1, h), br, :])
            vb = _b(bulk[_unit(2, h), br, :])
            if first:
                kv_sc[0, h] = _u(k)
                kv_sc[1, h] = _u(v)
                k = jnp.concatenate([k, kb], axis=0)
                v = jnp.concatenate([v, vb], axis=0)
            else:
                q = jnp.concatenate([q, _b(bulk[_unit(0, h), br, :])], axis=0)
                k = jnp.concatenate([k, kb, _b(kv_sc[0, h])], axis=0)
                v = jnp.concatenate([v, vb, _b(kv_sc[1, h])], axis=0)
            qkv[h] = (q, k, v)

        def qk(h):
            q, k, _ = qkv[h]
            s = jnp.where(mask, _dot_t(q, k) * SCALE, fill)
            p = jnp.exp(s - jnp.max(s, axis=-1, keepdims=True))
            den = jnp.sum(p, axis=-1, keepdims=True)
            ps[h] = (p * pl.reciprocal(den, approx=False)).astype(bf16)

        def pv(h):
            o = _dot(ps.pop(h), qkv.pop(h)[2])
            oall[0:nw // 2, h * 128:(h + 1) * 128] = _u(o.astype(bf16))

        side = list(side)
        for h in range(KSPLIT):
            proj_lo(h)
        for h in range(H):
            proj(h)
            if h - D1 >= 0:
                qk(h - D1)
            if h - D1 - D2 >= 0:
                pv(h - D1 - D2)
            if side and h >= 4 and h % 2 == 0:
                side.pop(0)()

        ka = (H - HB) * 128
        oa = _b(oall[0:nw // 2, 0:ka])
        accs = []
        nslot = D1 + D2 + 1
        for i in range(nslot):
            while len(accs) < (NC * (i + 1)) // nslot:
                accs.append(_dot(oa, _b(wo_s[len(accs), 0:ka // 2, :])))
            if i < D1:
                qk(H + i - D1)
            if i < D1 + D2:
                pv(H + i - D1 - D2)
        ob = _b(oall[0:nw // 2, ka:])
        res = [_dot(ob, _b(wo_s[j, ka // 2:, :])) + accs[j] for j in range(NC)]

        mem_sc[...] = jnp.concatenate([r[:M] for r in res], axis=1).astype(bf16).astype(f32)

        lo, n = (0, 24) if first else (24, 40)

        def mix(j):
            if first:
                bj = res[j][8:32]
            else:
                bj = jnp.concatenate([res[j][32:48], res[j][8:32]], axis=0)
            cols = slice(j * 128, (j + 1) * 128)
            aj = x_v[jp, lo:lo + n, cols].astype(f32) * ys[j, pl.ds(pl.multiple_of(jp * 64 + lo, 8), n), :]
            x_v[jp, lo:lo + n, cols] = (bj + gtab[jp, lo:lo + n, :] * (aj - bj)).astype(bf16)

        return [functools.partial(mix, j) for j in range(NC)]

    def pairs(jq, carry):
        epi = []
        for r in range(UN):
            for first in (True, False):
                epi = step(first, jq * UN + r, epi)
        _interleave(epi)
        rows = pl.ds(jq * UN, UN)
        pltpu.make_async_copy(x_v.at[rows], out_hbm.at[rows], sems.at[10]).start()
        return carry

    lax.fori_loop(0, NP // UN, pairs, 0)
    pltpu.make_async_copy(x_v, out_hbm, sems.at[10]).wait()


@functools.partial(jax.jit, static_argnames=("B_seg_len",))
def pallas_gated_mix__ssm_conv_h3__memory_aug_recurrent_mem_tr__prompt_kernel(
    A_q, A_k, A_v, A_shift_k, A_ssm_k, A_ssm_D, B_x, B_mem0, B_Wq, B_Wk, B_Wv, B_Wo,
    B_seg_len, gate_w,
):
    del B_x
    assert int(B_seg_len) == SEG and A_q.shape == (1, S, D) and B_Wq.shape == (D, H, E)
    fwd, inv = _dft_consts()
    out = pl.pallas_call(
        _kernel,
        out_shape=jax.ShapeDtypeStruct((NP, 64, D), bf16),
        in_specs=[pl.BlockSpec(memory_space=pl.ANY)] * 14,
        out_specs=pl.BlockSpec(memory_space=pl.ANY),
        scratch_shapes=[
            pltpu.VMEM((NP, 64, D), bf16),
            pltpu.VMEM((NP, 8, D), u32),
            pltpu.VMEM((NC, S + 64, 128), bf16),
            pltpu.VMEM((NC, S, 128), bf16),
            pltpu.VMEM((NC, 128, S), bf16),
            pltpu.VMEM((NW + 2, 2, D // 2, E), u32),
            pltpu.VMEM((3 * H + 4, D // 2, E), u32),
            pltpu.VMEM((NC, H * E // 2, 128), u32),
            pltpu.VMEM((3 * H, NP * 8, E), u32),
            pltpu.VMEM((NC + 1, S, 128), f32),
            pltpu.VMEM((NP, 64, 128), f32),
            pltpu.VMEM((S // 2, 128), u32),
            pltpu.VMEM((2, 128, 128), f32),
            pltpu.VMEM((3, NB, 128, 128), f32),
            pltpu.VMEM((3, NB, 128, 128), f32),
            pltpu.VMEM((NB, 256, 128), f32),
            pltpu.VMEM((M, D), f32),
            pltpu.VMEM((2, H, 16, E), u32),
            pltpu.VMEM((24, H * E), u32),
            pltpu.SMEM((1,), jnp.int32),
            pltpu.VMEM((KS, D), bf16), pltpu.VMEM((D,), bf16), pltpu.VMEM((D,), bf16),
            pltpu.VMEM((M, D), bf16), pltpu.VMEM((256, 128), u32), pltpu.VMEM((64, 128), u32),
            pltpu.VMEM((NC, KS, 128), f32), pltpu.VMEM((NC, 1, 128), f32), pltpu.VMEM((1, D), f32),
            pltpu.SemaphoreType.DMA((11,)),
        ],
        compiler_params=pltpu.CompilerParams(vmem_limit_bytes=126 * 1024 * 1024),
    )(
        A_q.reshape(NP, 64, D), A_k.reshape(S, D), A_v.reshape(S, D), A_ssm_k,
        B_Wq.reshape(D // 2, 2, H, E), B_Wk.reshape(D // 2, 2, H, E), B_Wv.reshape(D // 2, 2, H, E),
        B_Wo.reshape(H * E, D),
        A_shift_k.T, A_ssm_D, gate_w, B_mem0.reshape(M, D), jnp.asarray(fwd), jnp.asarray(inv),
    )
    return out.reshape(1, S, D)
```

```python
import functools

import jax
import jax.numpy as jnp
import numpy as np
from jax import lax
import jax.experimental.pallas as pl
import jax.experimental.pallas.tpu as pltpu

f32, bf16, u32 = jnp.float32, jnp.bfloat16, jnp.uint32

S, D, H, E, M, SEG, KS = 2048, 1024, 32, 128, 8, 32, 4
NP = S // (2 * SEG)
NC = D // 128
NB = S // 128
NW = 3 * H // 2
SCALE = float(E) ** -0.5
NEG = -1000000000.0
D1, D2, HB = 2, 2, 5
KSPLIT = 2
UN = 2
MB = 64


def _unit(which, h):
    pj = h // 2
    if which == 0:
        slot = pj if pj < 8 else 8 + 5 * (pj - 8)
    else:
        slot = 8 + 5 * (pj // 2) + (1 if which == 1 else 3) + pj % 2
    return 2 * slot + h % 2


def _pack_rows(a):
    b = np.asarray(a, np.float32).astype(jnp.bfloat16).view(np.uint16).astype(np.uint32)
    return b[0::2] | (b[1::2] << 16)


def _dft_consts():
    t = np.arange(128, dtype=np.float64)
    f = np.arange(128, dtype=np.float64) + 0.5
    phi = 2.0 * np.pi * f / 256.0
    tu = np.outer(phi, t)
    tk = np.outer(phi, t - 63.5)
    ti = np.outer(np.arange(64) + 0.5, phi)
    fwd = np.concatenate([np.cos(tu), -np.sin(tu), np.cos(tk), -np.sin(tk)], axis=0)
    inv = np.concatenate([np.cos(ti), np.sin(ti)], axis=0) / 128.0
    return _pack_rows(fwd), _pack_rows(inv)


def _b(x):
    return pltpu.bitcast(x, bf16)


def _u(x):
    return pltpu.bitcast(x, u32)


def _dot(a, b):
    return jnp.dot(a, b, preferred_element_type=f32)


def _dot_t(a, b):
    return lax.dot_general(a, b, (((1,), (1,)), ((), ())), preferred_element_type=f32)


def _cat(lists):
    return [f for lst in lists for f in lst]


def _interleave(*lists):
    items = []
    for li, lst in enumerate(lists):
        for i, fn in enumerate(lst):
            items.append(((i + 0.5) / len(lst), li, i, fn))
    items.sort(key=lambda t: t[:3])
    for it in items:
        it[3]()


def _kernel(x_hbm, k_hbm, v_hbm, ssm_hbm, wq_hbm, wk_hbm, wv_hbm, wo_hbm,
            shift_hbm, ssmd_hbm, gate_hbm, mem0_hbm, fwd_hbm, inv_hbm,
            out_hbm,
            x_v, xbp, k_v, v_v, ssm_v, wraw, w_s, wo_s, bulk,
            ys, gtab, kvb, kraw, uh, kh, zz, mem_sc, kv_sc, oall, flag,
            shift_v, ssmd_v, gate_v, mem0_ref, fwd_ref, inv_ref, shift_ref, ssmd_ref, gate_ref,
            sems):
    w32 = [w.bitcast(u32) for w in (wq_hbm, wk_hbm, wv_hbm)]
    wo32 = wo_hbm.bitcast(u32)
    x32 = x_hbm.bitcast(u32)

    def kv_copies(c, sem):
        return [
            pltpu.make_async_copy(k_hbm.at[:, pl.ds(c * 128, 128)], k_v.at[c, pl.ds(16, S), :], sem),
            pltpu.make_async_copy(v_hbm.at[:, pl.ds(c * 128, 128)], v_v.at[c], sem),
        ]

    def sx_copies(c):
        return [
            pltpu.make_async_copy(ssm_hbm.at[pl.ds(c * 128, 128), :], ssm_v.at[c], sems.at[8 + c % 2]),
            pltpu.make_async_copy(x_hbm.at[pl.ds(4 * c, 4)], x_v.at[pl.ds(4 * c, 4)], sems.at[8 + c % 2]),
        ]

    def kv_next(c):
        return kv_copies(c + 1, sems.at[8 + c % 2])

    def w_copy(which, pj, slot, sem):
        return [pltpu.make_async_copy(w32[which].at[:, par, pj, :], wraw.at[slot, par], sem) for par in range(2)]

    def single_copies(t):
        return w_copy(1, 0, 9, sems.at[1]) if t == 9 else w_copy(0, t, t, sems.at[t % 8])

    def single_wait(t):
        pltpu.make_async_copy(wraw.at[t], wraw.at[t], sems.at[t % 8]).wait()

    def group_lo(g):
        sem = sems.at[2 + g % 3]
        return (w_copy(1, 2 * g + 1, 10 + 5 * g, sem) + w_copy(2, 2 * g, 11 + 5 * g, sem)
                + w_copy(2, 2 * g + 1, 12 + 5 * g, sem))

    def group_hi(g):
        sem = sems.at[2 + g % 3]
        return w_copy(0, 9 + g, 13 + 5 * g, sem) + w_copy(1, 2 * g + 2, 14 + 5 * g, sem)

    def wo_copy(j):
        return pltpu.make_async_copy(wo32.at[:, pl.ds(j * 128, 128)], wo_s.at[j], sems.at[10])

    def xb_copy():
        return pltpu.make_async_copy(x32.at[:, pl.ds(12, 8), :], xbp, sems.at[8])

    def small_copies():
        return [pltpu.make_async_copy(a, b, sems.at[10]) for a, b in
                ((shift_hbm, shift_v), (ssmd_hbm, ssmd_v), (gate_hbm, gate_v), (mem0_hbm, mem0_ref),
                 (fwd_hbm, fwd_ref), (inv_hbm, inv_ref))] + kv_copies(0, sems.at[10])

    def start_all(cps):
        for cp in cps:
            cp.start()

    def wait_all(cps):
        for cp in cps:
            cp.wait()

    def start_head_batch(t):
        start_all({0: lambda: _cat(single_copies(u) for u in range(4, 8)),
                   2: lambda: sx_copies(0) + kv_next(0) + single_copies(8) + single_copies(9),
                   4: lambda: group_lo(0) + group_hi(0),
                   6: lambda: sx_copies(1) + kv_next(1) + group_lo(1) + group_hi(1)}[t]())

    def start_late_batch(i):
        g = i + 2
        cps = sx_copies(g) + (kv_next(g) if g < NC - 1 else []) + group_lo(g) + (group_hi(g) if g < NC - 1 else [])
        if i < NC // 2:
            cps += [wo_copy(2 * i), wo_copy(2 * i + 1)]
        start_all(cps)

    def once_if(cond, fn):
        def body(_, carry):
            fn()
            return carry
        lax.fori_loop(0, cond.astype(jnp.int32), body, 0)

    start_all(single_copies(0) + [xb_copy()] + _cat(single_copies(u) for u in range(1, 4)) + small_copies())

    flag[0] = 1
    for c in range(NC):
        k_v[c, 0:16, :] = jnp.zeros((16, 128), bf16)

    ra = lax.broadcasted_iota(jnp.int32, (32, 48), 0)
    ca = lax.broadcasted_iota(jnp.int32, (32, 48), 1)
    same_a = ca < 40
    mask_a = same_a & ((ra < M) | (ra >= ca))
    rb = lax.broadcasted_iota(jnp.int32, (48, 80), 0)
    cb = lax.broadcasted_iota(jnp.int32, (48, 80), 1)
    q_in_a = (rb >= 32) & (rb < 40)
    k_in_a = ((cb >= 32) & (cb < 40)) | (cb >= 48)
    qpos = jnp.where(rb < 8, rb, jnp.where(rb < 32, rb + 8, jnp.where(rb < 40, rb, rb - 32)))
    kpos = jnp.where(cb < 8, cb, jnp.where(cb < 32, cb + 8,
                     jnp.where(cb < 40, cb, jnp.where(cb < 48, cb - 32, cb - 48))))
    same_b = q_in_a == k_in_a
    mask_b = same_b & ((qpos < M) | (qpos >= kpos))
    fill_a = jnp.where(same_a, NEG, -jnp.inf).astype(f32)
    fill_b = jnp.where(same_b, NEG, -jnp.inf).astype(f32)

    def pre(c, ys_c, b, n=128):
        r0 = b * n if isinstance(b, int) else pl.multiple_of(b * n, n)
        h0 = b * (n // 2) if isinstance(b, int) else pl.multiple_of(b * (n // 2), n // 2)
        sh = shift_ref[c]
        kx = k_v[c, pl.ds(r0, n + 16), :].astype(f32)[8:]
        ks = kx[8:] * sh[0:1, :]
        for j in range(1, KS):
            ks = ks + kx[8 - j:8 + n - j] * sh[j:j + 1, :]
        kv = (ks * v_v[c, pl.ds(r0, n), :].astype(f32)).astype(bf16)
        ys_c[pl.ds(r0, n), :] = kv.astype(f32) * ssmd_ref[c]
        kvb[pl.ds(h0, n // 2), :] = _u(kv)

    def fwd_thunks(c, cn, ys_n):
        def fu(i):
            kv = _b(kvb[64 * i:64 * (i + 1), :])
            ur = _dot(_b(fwd_ref[0:64, :]), kv)
            ui = _dot(_b(fwd_ref[64:128, :]), kv)
            uh[0, i] = ur
            uh[1, i] = ui
            uh[2, i] = ur + ui

        def fk(i):
            kb = ssm_v[c, :, 128 * i:128 * (i + 1)]
            kr = _dot_t(_b(fwd_ref[128:192, :]), kb)
            ki = _dot_t(_b(fwd_ref[192:256, :]), kb)
            if i == 0:
                pr, pi = kr, ki
            else:
                row = lax.broadcasted_iota(jnp.int32, (128, 128), 0)
                sgn = jnp.where(row % 2 == 0, 1.0, -1.0).astype(f32)
                pr = kr - sgn * kraw[1]
                pi = ki + sgn * kraw[0]
            kraw[0] = kr
            kraw[1] = ki
            kh[0, i] = pr
            kh[1, i] = pi
            kh[2, i] = pr + pi

        return _cat([functools.partial(fu, i), functools.partial(fk, i), functools.partial(pre, cn, ys_n, i)]
                    for i in range(NB))

    def group4(comp, rows, b):
        acc = None
        for j in range(4 * b + 4):
            lo = max(0, j - 4 * b)
            t = kh[comp, 4 * b + lo - j:4 * b + 4 - j, rows, :] * uh[comp, j, rows, :][None]
            if acc is None:
                acc = t
            elif lo == 0:
                acc = acc + t
            else:
                acc = jnp.concatenate([acc[:lo], acc[lo:] + t], axis=0)
        return acc

    def mac_thunks(p):
        rows, rows2 = pl.ds(8 * p, 8), pl.ds(128 + 8 * p, 8)
        out = []
        for b in range(4):
            st = {}

            def f0(b=b, st=st):
                st['a'] = group4(0, rows, b)

            def f1(b=b, st=st):
                bb = group4(1, rows, b)
                a = st.pop('a')
                zz[4 * b:4 * b + 4, rows, :] = a - bb
                st['ab'] = a + bb

            def f2(b=b, st=st):
                zz[4 * b:4 * b + 4, rows2, :] = group4(2, rows, b) - st.pop('ab')

            out += [f0, f1, f2]
        return out

    def inv_thunks(ys_c):
        def f(i):
            a = _dot(_b(inv_ref[0:32, :]), zz[i, 0:128, :].astype(bf16))
            b = _dot(_b(inv_ref[32:64, :]), zz[i, 128:256, :].astype(bf16))
            lo = a + b
            rev = 7 - lax.broadcasted_iota(jnp.int32, (8, 128), 0)
            y = jnp.concatenate(
                [jnp.take_along_axis(lo[8 * r:8 * r + 8], rev, axis=0) for r in range(7, -1, -1)] + [a - b],
                axis=0)
            ys_c[128 * i:128 * (i + 1), :] = ys_c[128 * i:128 * (i + 1), :] + y.astype(bf16).astype(f32)
        return [functools.partial(f, i) for i in range(NB)]

    def gate_thunks(i):
        def f(r):
            rows = pl.ds(32 * (r % 2), 32)
            xo = x_v[4 * i + r // 2, rows, :].astype(f32)
            g = jax.nn.sigmoid(jnp.sum(xo * gate_ref[...], axis=-1, keepdims=True))
            gtab[4 * i + r // 2, rows, :] = jnp.broadcast_to(g, (32, 128))
        return [functools.partial(f, r) for r in range(8)]

    def repack_thunks(src, dst):
        def f(db):
            r = pl.ds(db * 64, 64)
            ev, od = src[0, r, :], src[1, r, :]
            dst[0, r, :] = (ev & jnp.uint32(0xFFFF)) | (od << 16)
            dst[1, r, :] = (ev >> 16) | (od & jnp.uint32(0xFFFF0000))
        return [functools.partial(f, db) for db in range(8)]

    def bulk_thunks(wsrc, dst, nk=1):
        st = {}

        def f(mc, kk):
            kw = D // nk
            lhs = xbp[mc * (MB // 16):(mc + 1) * (MB // 16), :, kk * kw:(kk + 1) * kw].reshape(MB // 2, kw)
            r = _dot(_b(lhs), _b(wsrc[kk * kw // 2:(kk + 1) * kw // 2, :]))
            if kk > 0:
                r = r + st.pop(mc)
            if kk < nk - 1:
                st[mc] = r
            else:
                dst[mc * (MB // 2):(mc + 1) * (MB // 2), :] = _u(r.astype(bf16))
        return [functools.partial(f, mc, kk) for mc in range(NP * 16 // MB) for kk in range(nk)]

    single_wait(0)
    _interleave(repack_thunks(wraw.at[0], w_s.at[pl.ds(0, 2)]))
    xb_copy().wait()

    start_head_batch(0)

    @pl.when(flag[0] > 0)
    def _():
        _interleave(_cat(bulk_thunks(w_s.at[u], bulk.at[u]) for u in range(2)))

    single_wait(1)
    _interleave(repack_thunks(wraw.at[1], w_s.at[pl.ds(2, 2)]))

    def head(with_pre, t, carry):
        for c in ((4,) if with_pre else (2,)):
            once_if(t == c, functools.partial(start_head_batch, c))
        single_wait(t + 1)
        wwin = w_s.at[pl.ds(t * 2, 4)]
        bwin = bulk.at[pl.ds(t * 2, 2)]

        @pl.when(flag[0] > 0)
        def _():
            lists = [_cat(bulk_thunks(wwin.at[u], bwin.at[u]) for u in range(2)),
                     repack_thunks(wraw.at[t + 1], wwin.at[pl.ds(2, 2)])]
            if with_pre:
                lists.append([functools.partial(pre, 0, ys.at[0], 8 * (t - 4) + b, 64) for b in range(8)])
            _interleave(*lists)
        return carry

    lax.fori_loop(1, 4, functools.partial(head, False), 0)
    wait_all(small_copies())
    sh32 = shift_v[...].astype(f32)
    sd32 = ssmd_v[...].reshape(1, D).astype(f32)
    for c in range(NC):
        shift_ref[c] = sh32[:, c * 128:(c + 1) * 128]
        ssmd_ref[c] = sd32[:, c * 128:(c + 1) * 128]
    gate_ref[...] = gate_v[...].reshape(1, D).astype(f32)
    mem_sc[...] = mem0_ref[...].astype(f32)
    lax.fori_loop(4, 8, functools.partial(head, True), 0)
    single_wait(9)
    _interleave(repack_thunks(wraw.at[9], w_s.at[pl.ds(18, 2)]))
    wait_all(sx_copies(0) + kv_next(0))
    start_head_batch(6)

    def block_b(i):
        first = isinstance(i, int)
        wwin = w_s.at[pl.ds(16 + i * 10, 2)]
        bwin = bulk.at[pl.ds(16 + i * 10, 2)]
        ywin = ys.at[pl.ds(0 if first else i - 1, 3)]
        lists = [_cat(bulk_thunks(wwin.at[u], bwin.at[u]) for u in range(2)),
                 fwd_thunks(i, 1 if first else jnp.minimum(i + 1, NC - 1), ywin.at[1 if first else 2]),
                 gate_thunks(i)]
        if not first:
            lists.insert(2, inv_thunks(ywin.at[0]))
        _interleave(*lists)

    @pl.when(flag[0] > 0)
    def _():
        block_b(0)

    def pro(i, carry):
        wwin = w_s.at[pl.ds(18 + i * 10, 12)]
        bwin = bulk.at[pl.ds(18 + i * 10, 8)]
        rwin = wraw.at[pl.ds(10 + i * 5, 5)]
        gsem = sems.at[2 + i % 3]

        @pl.when(i < NC - 1)
        def _():
            pltpu.make_async_copy(rwin, rwin, gsem).wait()

        @pl.when(i == NC - 1)
        def _():
            pltpu.make_async_copy(rwin.at[0:3], rwin.at[0:3], gsem).wait()

        for c in range(NC - 2):
            once_if(i == c, functools.partial(start_late_batch, c))

        @pl.when(flag[0] > 0)
        def _():
            _interleave(_cat(bulk_thunks(wwin.at[u], bwin.at[u], 2) for u in range(8)),
                        _cat(mac_thunks(p) for p in range(16)),
                        _cat(repack_thunks(rwin.at[t], wwin.at[pl.ds(2 + 2 * t, 2)]) for t in range(5)))

        @pl.when(i < NC - 1)
        def _():
            wait_all(sx_copies(jnp.minimum(i + 1, NC - 1)))

        @pl.when(i < NC - 2)
        def _():
            wait_all(kv_next(jnp.minimum(i + 1, NC - 2)))

        @pl.when(i < NC - 1)
        def _():
            block_b(jnp.minimum(i + 1, NC - 1))
        return carry

    lax.fori_loop(0, NC, pro, 0)
    _interleave(inv_thunks(ys.at[NC - 1]))
    wait_all([wo_copy(j) for j in range(NC)])

    def step(first, jp, side):
        xr = x_v[jp, 0:24, :] if first else x_v[jp, 40:64, :]
        lhs = jnp.concatenate([mem_sc[...], xr.astype(f32)], axis=0).astype(bf16)
        nw = 32 if first else 48
        mask, fill = (mask_a, fill_a) if first else (mask_b, fill_b)
        br = pl.ds(pl.multiple_of(jp * 8, 8), 8)
        qkv, ps, part = {}, {}, {}

        def proj_lo(h):
            part[h] = [_dot(lhs[:, :D // 2], _b(w_s[_unit(t, h), 0:D // 4, :])) for t in range(3)]

        def proj(h):
            if h in part:
                low = part.pop(h)
                v, k, q = [(_dot(lhs[:, D // 2:], _b(w_s[_unit(t, h), D // 4:, :])) + low[t]).astype(bf16)
                           for t in (2, 1, 0)]
            else:
                v, k, q = [_dot(lhs, _b(w_s[_unit(t, h)])).astype(bf16) for t in (2, 1, 0)]
            kb = _b(bulk[_unit(1, h), br, :])
            vb = _b(bulk[_unit(2, h), br, :])
            if first:
                kv_sc[0, h] = _u(k)
                kv_sc[1, h] = _u(v)
                k = jnp.concatenate([k, kb], axis=0)
                v = jnp.concatenate([v, vb], axis=0)
            else:
                q = jnp.concatenate([q, _b(bulk[_unit(0, h), br, :])], axis=0)
                k = jnp.concatenate([k, kb, _b(kv_sc[0, h])], axis=0)
                v = jnp.concatenate([v, vb, _b(kv_sc[1, h])], axis=0)
            qkv[h] = (q, k, v)

        def qk(h):
            q, k, _ = qkv[h]
            s = jnp.where(mask, _dot_t(q, k) * SCALE, fill)
            p = jnp.exp(s - jnp.max(s, axis=-1, keepdims=True))
            den = jnp.sum(p, axis=-1, keepdims=True)
            ps[h] = (p * pl.reciprocal(den, approx=False)).astype(bf16)

        def pv(h):
            o = _dot(ps.pop(h), qkv.pop(h)[2])
            oall[0:nw // 2, h * 128:(h + 1) * 128] = _u(o.astype(bf16))

        side = list(side)
        for h in range(KSPLIT):
            proj_lo(h)
        for h in range(H):
            proj(h)
            if h - D1 >= 0:
                qk(h - D1)
            if h - D1 - D2 >= 0:
                pv(h - D1 - D2)
            if side and h >= 2 and h % 2 == 0:
                side.pop(0)()

        ka = (H - HB) * 128
        oa = _b(oall[0:nw // 2, 0:ka])
        accs = []
        nslot = D1 + D2 + 1
        for i in range(nslot):
            while len(accs) < (NC * (i + 1)) // nslot:
                accs.append(_dot(oa, _b(wo_s[len(accs), 0:ka // 2, :])))
            if i < D1:
                qk(H + i - D1)
            if i < D1 + D2:
                pv(H + i - D1 - D2)
        ob = _b(oall[0:nw // 2, ka:])
        res = [_dot(ob, _b(wo_s[j, ka // 2:, :])) + accs[j] for j in range(NC)]

        mem_sc[...] = jnp.concatenate([r[:M] for r in res], axis=1).astype(bf16).astype(f32)

        lo, n = (0, 24) if first else (24, 40)

        def mix(j):
            if first:
                bj = res[j][8:32]
            else:
                bj = jnp.concatenate([res[j][32:48], res[j][8:32]], axis=0)
            cols = slice(j * 128, (j + 1) * 128)
            aj = x_v[jp, lo:lo + n, cols].astype(f32) * ys[j, pl.ds(pl.multiple_of(jp * 64 + lo, 8), n), :]
            x_v[jp, lo:lo + n, cols] = (bj + gtab[jp, lo:lo + n, :] * (aj - bj)).astype(bf16)

        return [functools.partial(mix, j) for j in range(NC)]

    def pairs(jq, carry):
        epi = []
        for r in range(UN):
            for first in (True, False):
                epi = step(first, jq * UN + r, epi)
        _interleave(epi)
        rows = pl.ds(jq * UN, UN)
        pltpu.make_async_copy(x_v.at[rows], out_hbm.at[rows], sems.at[10]).start()
        return carry

    lax.fori_loop(0, NP // UN, pairs, 0)
    pltpu.make_async_copy(x_v, out_hbm, sems.at[10]).wait()


@functools.partial(jax.jit, static_argnames=("B_seg_len",))
def pallas_gated_mix__ssm_conv_h3__memory_aug_recurrent_mem_tr__prompt_kernel(
    A_q, A_k, A_v, A_shift_k, A_ssm_k, A_ssm_D, B_x, B_mem0, B_Wq, B_Wk, B_Wv, B_Wo,
    B_seg_len, gate_w,
):
    del B_x
    assert int(B_seg_len) == SEG and A_q.shape == (1, S, D) and B_Wq.shape == (D, H, E)
    fwd, inv = _dft_consts()
    out = pl.pallas_call(
        _kernel,
        out_shape=jax.ShapeDtypeStruct((NP, 64, D), bf16),
        in_specs=[pl.BlockSpec(memory_space=pl.ANY)] * 14,
        out_specs=pl.BlockSpec(memory_space=pl.ANY),
        scratch_shapes=[
            pltpu.VMEM((NP, 64, D), bf16),
            pltpu.VMEM((NP, 8, D), u32),
            pltpu.VMEM((NC, S + 64, 128), bf16),
            pltpu.VMEM((NC, S, 128), bf16),
            pltpu.VMEM((NC, 128, S), bf16),
            pltpu.VMEM((NW + 2, 2, D // 2, E), u32),
            pltpu.VMEM((3 * H + 4, D // 2, E), u32),
            pltpu.VMEM((NC, H * E // 2, 128), u32),
            pltpu.VMEM((3 * H, NP * 8, E), u32),
            pltpu.VMEM((NC + 1, S, 128), f32),
            pltpu.VMEM((NP, 64, 128), f32),
            pltpu.VMEM((S // 2, 128), u32),
            pltpu.VMEM((2, 128, 128), f32),
            pltpu.VMEM((3, NB, 128, 128), f32),
            pltpu.VMEM((3, NB, 128, 128), f32),
            pltpu.VMEM((NB, 256, 128), f32),
            pltpu.VMEM((M, D), f32),
            pltpu.VMEM((2, H, 16, E), u32),
            pltpu.VMEM((24, H * E), u32),
            pltpu.SMEM((1,), jnp.int32),
            pltpu.VMEM((KS, D), bf16), pltpu.VMEM((D,), bf16), pltpu.VMEM((D,), bf16),
            pltpu.VMEM((M, D), bf16), pltpu.VMEM((256, 128), u32), pltpu.VMEM((64, 128), u32),
            pltpu.VMEM((NC, KS, 128), f32), pltpu.VMEM((NC, 1, 128), f32), pltpu.VMEM((1, D), f32),
            pltpu.SemaphoreType.DMA((11,)),
        ],
        compiler_params=pltpu.CompilerParams(vmem_limit_bytes=126 * 1024 * 1024),
    )(
        A_q.reshape(NP, 64, D), A_k.reshape(S, D), A_v.reshape(S, D), A_ssm_k,
        B_Wq.reshape(D // 2, 2, H, E), B_Wk.reshape(D // 2, 2, H, E), B_Wv.reshape(D // 2, 2, H, E),
        B_Wo.reshape(H * E, D),
        A_shift_k.T, A_ssm_D, gate_w, B_mem0.reshape(M, D), jnp.asarray(fwd), jnp.asarray(inv),
    )
    return out.reshape(1, S, D)
```
